```python
import os as _os
_os.environ.setdefault("JAX_PLATFORMS", "cpu")
import jax
import jax.numpy as jnp

def _softmax(x, axis=-1):
    return jax.nn.softmax(x, axis=axis)
def _gelu(x):
    return jax.nn.gelu(x, approximate=True)
def _silu(x):
    return jax.nn.silu(x)
def _sigmoid(x):
    return jax.nn.sigmoid(x)
def _layernorm(x, axis=-1, eps=1e-5):
    m = jnp.mean(x, axis=axis, keepdims=True)
    v = jnp.var(x, axis=axis, keepdims=True)
    return (x - m) / jnp.sqrt(v + eps)
def _scatter_add(tgt, idx, src, axis=0):
    return tgt.at[idx].add(src)
def _segment_sum(src, seg, n):
    return jax.ops.segment_sum(src, seg, n)
class _Rng:
    def __init__(self, key):
        self._k = key
    def _next(self):
        self._k, sub = jax.random.split(self._k)
        return sub
    def normal(self, shape):
        return jax.random.normal(self._next(), shape, dtype=jnp.bfloat16)
    def randint(self, lo, hi, shape):
        return jax.random.randint(self._next(), shape, lo, hi, dtype=jnp.int32)
    def uniform(self, shape, lo=0.0, hi=1.0):
        return jax.random.uniform(self._next(), shape, jnp.bfloat16, lo, hi)
    def permutation(self, n):
        return jax.random.permutation(self._next(), n)


kernel_name = 'parallel_sum__mha_block__swiglu_ffn__prompt'

def setup_inputs():
    _rng = _Rng(jax.random.key(int.from_bytes(__import__("os").urandom(4), "little")))
    _w = (lambda a: (lambda t: t.astype(jnp.bfloat16) if jnp.issubdtype(t.dtype, jnp.floating) else t)(jnp.asarray(a)))
    def _A_setup():
        B, S, D, H = 1, 2048, 640, 32
        return {
            "x": _w((lambda *s: _rng.normal(s) * 0.05)(B, S, D)),
            "wqkv": _w((lambda *s: _rng.normal(s) * 0.1)(D, 3 * D)),
            "wo": _w((lambda *s: _rng.normal(s) * 0.05)(D, D)),
        }
    _A_in = _A_setup()

    def _B_setup():
        B, S, D, F = 1, 2048, 640, 1536
        return {
            "x": _w((lambda *s: _rng.normal(s) * 0.05)(B, S, D)),
            "w_gate": _w((lambda *s: _rng.normal(s) * 0.05)(D, F)),
            "w_up": _w((lambda *s: _rng.normal(s) * 0.05)(D, F)),
            "w_down": _w((lambda *s: _rng.normal(s) * 0.05)(F, D)),
        }
    _B_in = _B_setup()

    return {
        "A_x": _A_in["x"],
        "A_wqkv": _A_in["wqkv"],
        "A_wo": _A_in["wo"],
        "B_x": _B_in["x"],
        "B_w_gate": _B_in["w_gate"],
        "B_w_up": _B_in["w_up"],
        "B_w_down": _B_in["w_down"],
    }

def reference(A_x, A_wqkv, A_wo, B_x, B_w_gate, B_w_up, B_w_down):
    def _A_ref(x, wqkv, wo):
        B, S, D = x.shape
        H = 32
        Dh = D // H
        qkv = (lambda x, *d: x.transpose(*d))((x @ wqkv).reshape(B, S, 3, H, Dh), 2, 0, 3, 1, 4)
        q, k, v = qkv[0], qkv[1], qkv[2]
        scores = jnp.einsum("bhqd,bhkd->bhqk", q, k) * (Dh ** -0.5)
        p = _softmax(scores, axis=-1)
        o = jnp.einsum("bhqk,bhkd->bhqd", p, v)
        return (lambda x, *d: x.transpose(*d))(o, 0, 2, 1, 3).reshape(B, S, D) @ wo

    def _B_ref(x, w_gate, w_up, w_down):
        g = _silu(x @ w_gate)
        u = x @ w_up
        return (g * u) @ w_down

    x = A_x
    xn = _layernorm(x, axis=-1)
    return x + _A_ref(xn, A_wqkv, A_wo) + _B_ref(xn, B_w_gate, B_w_up, B_w_down)
```

```python
import functools
import math

import jax
import jax.numpy as jnp
import jax.experimental.pallas as pl
import jax.experimental.pallas.tpu as pltpu

S = 2048
D = 640
H = 32
DH = 20
F = 1536
EPS = 1e-5
NSLAB = 6
SLAB_OFF = (0, 120, 240, 360, 480, 512)
LOG2E = 1.4426950408889634

TQ = 512
CK = 128
NCK = S // CK
NQ = S // TQ
RC = 512
FC = 512
SKEW = 2


def _kernel(x_ref, wqkv_ref, wo_ref, wg_ref, wu_ref, wd_ref, o_ref,
            xn_s, wk_s, wqvt_s, k_s, qm_s, vt_s, s_a, s_b, ot_s):
    step = pl.program_id(0)
    f32 = jnp.float32
    bf16 = jnp.bfloat16

    @pl.when(step == 0)
    def _prologue():
        for j in range(NSLAB):
            wk_s[:, j * 128:(j + 1) * 128] = wqkv_ref[:, D + SLAB_OFF[j]: D + SLAB_OFF[j] + 128]
        wqvt_s[0:D, :] = wqkv_ref[:, 0:D].T
        wqvt_s[D:2 * D, :] = wqkv_ref[:, 2 * D:3 * D].T

        def chunk(r, carry):
            rows = pl.ds(pl.multiple_of(r * RC, RC), RC)
            x = x_ref[rows, :].astype(f32)
            mu = jnp.mean(x, axis=-1, keepdims=True)
            xc = x - mu
            var = jnp.mean(xc * xc, axis=-1, keepdims=True)
            xn = (xc * jax.lax.rsqrt(var + EPS)).astype(bf16)
            xn_s[rows, :] = xn
            kk = jnp.dot(xn, wk_s[...], preferred_element_type=f32).astype(bf16)
            for j in range(NSLAB):
                k_s[j, rows, :] = kk[:, j * 128:(j + 1) * 128]
            qt = jax.lax.dot_general(wqvt_s[0:D, :], xn, (((1,), (1,)), ((), ())),
                                     preferred_element_type=f32) * (DH ** -0.5 * LOG2E)
            row128 = jax.lax.broadcasted_iota(jnp.int32, (128, RC), 0)
            for h in range(H):
                off = SLAB_OFF[h // 6]
                lo = DH * h - off
                blk = qt[off:off + 128, :]
                qm_s[r, h] = jnp.where((row128 >= lo) & (row128 < lo + DH), blk, 0.0).astype(bf16)
            vt = jax.lax.dot_general(wqvt_s[D:2 * D, :], xn, (((1,), (1,)), ((), ())),
                                     preferred_element_type=f32)
            vt = vt.astype(bf16).astype(f32)
            row24 = jax.lax.broadcasted_iota(jnp.int32, (24, RC), 0)
            for h in range(H):
                base = (DH * h // 8) * 8
                ones_row = 20 if h % 2 == 0 else 0
                vt_s[r, h] = jnp.where(row24 == ones_row, 1.0, vt[base:base + 24, :])
            return carry

        jax.lax.fori_loop(0, S // RC, chunk, 0)

    def qk_chunk(h, s_s, c, m):
        s = jnp.dot(k_s[h // 6, pl.ds(c * CK, CK), :], qm_s[step, h], preferred_element_type=f32)
        s_s[pl.ds(c * CK, CK), :] = s
        mm = jnp.max(s.reshape(CK // 8, 8, TQ), axis=0)
        return mm if m is None else jnp.maximum(m, mm)

    def sm_chunk(h, s_s, c, m, acc):
        s = s_s[pl.ds(c * CK, CK), :]
        p = jnp.exp2(s - m).astype(bf16)
        kc = c * CK
        o = jnp.dot(vt_s[kc // RC, h, :, pl.ds(kc % RC, CK)], p, preferred_element_type=f32)
        return o if acc is None else acc + o

    def finish(g, parity, acc):
        ones_row = 20 if parity == 0 else 0
        l = acc[ones_row:ones_row + 1, :]
        o = acc * (1.0 / l)
        if parity == 0:
            ot_s[pl.ds(pl.multiple_of(40 * g, 8), 24), :] = o
        else:
            r0 = pl.multiple_of(40 * g + 16, 8)
            prev = ot_s[pl.ds(r0, 8), :]
            row8 = jax.lax.broadcasted_iota(jnp.int32, (8, TQ), 0)
            ot_s[pl.ds(r0, 8), :] = jnp.where(row8 < 4, prev, o[0:8, :])
            ot_s[pl.ds(r0 + 8, 16), :] = o[8:24, :]

    def stage(g, parity, hn, s_cur, s_nxt, m_cur):
        h = 2 * g + parity
        m = None
        acc = None
        for c in range(NCK):
            m = qk_chunk(hn, s_nxt, c, m)
            acc = sm_chunk(h, s_cur, c, m_cur, acc)
        finish(g, parity, acc)
        return jnp.max(m, axis=0, keepdims=True)

    m = None
    for c in range(NCK):
        m = qk_chunk(0, s_a, c, m)
    m0 = jnp.max(m, axis=0, keepdims=True)

    def body(g, m_cur):
        m1 = stage(g, 0, 2 * g + 1, s_a, s_b, m_cur)
        m2 = stage(g, 1, jnp.minimum(2 * g + 2, H - 1), s_b, s_a, m1)
        return m2

    jax.lax.fori_loop(0, H // 2, body, m0)

    rows = pl.ds(pl.multiple_of(step * TQ, TQ), TQ)
    acc = x_ref[rows, :].astype(f32)
    acc = acc + jax.lax.dot_general(ot_s[...].astype(bf16), wo_ref[...], (((0,), (0,)), ((), ())),
                                    preferred_element_type=f32)
    xn = xn_s[rows, :]
    for fc in range(F // FC):
        cols = slice(fc * FC, (fc + 1) * FC)
        g = jnp.dot(xn, wg_ref[:, cols], preferred_element_type=f32)
        u = jnp.dot(xn, wu_ref[:, cols], preferred_element_type=f32)
        hh = (g * jax.nn.sigmoid(g) * u).astype(bf16)
        acc = acc + jnp.dot(hh, wd_ref[cols, :], preferred_element_type=f32)
    o_ref[...] = acc.astype(o_ref.dtype)


@jax.jit
def pallas_parallel_sum__mha_block__swiglu_ffn__prompt_kernel(A_x, A_wqkv, A_wo, B_x, B_w_gate, B_w_up, B_w_down):
    x = A_x.reshape(S, D)
    bf16 = jnp.bfloat16
    f32 = jnp.float32
    full = lambda shape: pl.BlockSpec(shape, lambda i: (0,) * len(shape))
    out = pl.pallas_call(
        _kernel,
        grid=(NQ,),
        in_specs=[full((S, D)), full((D, 3 * D)), full((D, D)), full((D, F)), full((D, F)), full((F, D))],
        out_specs=pl.BlockSpec((TQ, D), lambda i: (i, 0)),
        out_shape=jax.ShapeDtypeStruct((S, D), bf16),
        scratch_shapes=[
            pltpu.VMEM((S, D), bf16),
            pltpu.VMEM((D, NSLAB * 128), bf16),
            pltpu.VMEM((2 * D, D), bf16),
            pltpu.VMEM((NSLAB, S, 128), bf16),
            pltpu.VMEM((NQ, H, 128, TQ), bf16),
            pltpu.VMEM((S // RC, H, 24, RC), f32),
            pltpu.VMEM((S, TQ), f32),
            pltpu.VMEM((S, TQ), f32),
            pltpu.VMEM((D, TQ), f32),
        ],
        compiler_params=pltpu.CompilerParams(
            dimension_semantics=("arbitrary",),
            vmem_limit_bytes=110 * 1024 * 1024),
        name="fused_block",
    )(x, A_wqkv, A_wo, B_w_gate, B_w_up, B_w_down)
    return out.reshape(1, S, D)
```

```python
import os

import jax
import jax.numpy as jnp
import jax.experimental.pallas as pl
import jax.experimental.pallas.tpu as pltpu

S = 2048
D = 640
H = 32
DH = 20
F = 1536
EPS = 1e-5
NSLAB = 6
SLAB_OFF = (0, 120, 240, 360, 480, 512)
ONES_LANE = (127, 127, 127, 127, 127, 0)
LOG2E = 1.4426950408889634
SHIFT = 100.0
L_MIN = 2.0 ** -80
L_MAX = 2.0 ** 120

TQ = 512
CK = 128
NCK = S // CK
NQ = S // TQ
RC = 512
NR = S // RC
FC = 512
_e = lambda k, d: int(os.environ.get(k, d))
TT = _e('TT', 256)
NB = _e('NB', 16)
NT = _e('NT', 1)
NTOK = 8
GATE = 19
LAGU = 2
LEAD = 1
NPB = 8
NBAT = _e('NBAT', 4)
FORCE_FB = _e('FORCE_FB', 0)

NGRP = [((c + 1) * NB) // NCK - (c * NB) // NCK for c in range(NCK)]
GBASE = [(c * NB) // NCK for c in range(NCK)]
UPH = NQ * NCK
BPI = NB * (4 // NT)
TPI = NCK * NTOK
BLIST = [(c, j, t0) for c in range(NCK) for j in range(NGRP[c]) for t0 in range(0, 4, NT)]
CPR = RC // CK


def _kernel(x_hbm, wqkv_hbm, wo_hbm, wg_hbm, wu_hbm, wd_hbm, o_hbm,
            x_s, wq_s, wkr_s, wv_s, wo_s, wg_s, wu_s, wd_s, out_s,
            xn_s, wk_s, wqvt_s, k_s, qm_s, vt_s, oraw_s, koff_s, qw_s, kb_a, kb_b,
            zero_s, acc_s, sfb_s, p0, p1, p2, p3, p4, p5, p6, p7, sem_in, sem_out):
    f32 = jnp.float32
    bf16 = jnp.bfloat16
    u32 = jnp.uint32
    i32 = jnp.int32
    pbufs = (p0, p1, p2, p3, p4, p5, p6, p7)
    kbuf = (kb_a, kb_b)

    cp_x0 = pltpu.make_async_copy(x_hbm.at[pl.ds(0, RC), :], x_s.at[pl.ds(0, RC), :], sem_in.at[0])
    cp_wk = pltpu.make_async_copy(wqkv_hbm.at[:, pl.ds(D, D)], wkr_s, sem_in.at[1])
    cp_wq = pltpu.make_async_copy(wqkv_hbm.at[:, pl.ds(0, D)], wq_s, sem_in.at[2])
    cp_wv = pltpu.make_async_copy(wqkv_hbm.at[:, pl.ds(2 * D, D)], wv_s, sem_in.at[3])
    cp_xr = pltpu.make_async_copy(x_hbm.at[pl.ds(RC, S - RC), :], x_s.at[pl.ds(RC, S - RC), :], sem_in.at[4])
    late = [pltpu.make_async_copy(src, dst, sem_in.at[5 + i])
            for i, (src, dst) in enumerate(((wo_hbm, wo_s), (wg_hbm, wg_s), (wu_hbm, wu_s), (wd_hbm, wd_s)))]
    cp_x0.start()
    cp_wk.start()
    cp_xr.start()
    cp_wq.start()
    cp_wv.start()

    def ln(r):
        rows = pl.ds(r * RC, RC)
        x = x_s[rows, :].astype(f32)
        mu = jnp.mean(x, axis=-1, keepdims=True)
        xc = x - mu
        var = jnp.mean(xc * xc, axis=-1, keepdims=True)
        xn_s[rows, :] = (xc * jax.lax.rsqrt(var + EPS)).astype(bf16)

    def ind_k():
        l = jax.lax.broadcasted_iota(i32, (NSLAB * 128, 128), 0)
        h = jax.lax.broadcasted_iota(i32, (NSLAB * 128, 128), 1)
        j = jnp.minimum(h // 6, 5)
        start = j * 128 + DH * h - jnp.where(j < 5, 120 * j, SLAB_OFF[5])
        return jnp.where((l >= start) & (l < start + DH) & (h < H), 1.0, 0.0).astype(bf16)

    def ind_q():
        h = jax.lax.broadcasted_iota(i32, (H, D), 0)
        d = jax.lax.broadcasted_iota(i32, (H, D), 1)
        return jnp.where((d >= DH * h) & (d < DH * h + DH), 1.0, 0.0).astype(bf16)

    def kproj(r, kmax):
        xn = xn_s[pl.ds(r * RC, RC), :]
        kk = jnp.dot(xn, wk_s[...], preferred_element_type=f32)
        k2 = kk * kk
        k2 = jnp.maximum(k2[0:RC // 2], k2[RC // 2:RC]).astype(bf16)
        kn2 = jnp.dot(k2, ind_k(), preferred_element_type=f32)
        kn2 = jnp.max(kn2.reshape(RC // 16, 8, 128), axis=0)
        kmax = kn2 if kmax is None else jnp.maximum(kmax, kn2)
        lane = jax.lax.broadcasted_iota(i32, (RC, 128), 1)
        for j in range(NSLAB):
            kj = jnp.where(lane == ONES_LANE[j], 1.0, kk[:, j * 128:(j + 1) * 128]).astype(bf16)
            k_s[j, pl.ds(r * (RC // 2), RC // 2), :] = pltpu.bitcast(kj, u32)
        if NB:
            rows = []
            for cc in range(CPR):
                c = r * CPR + cc
                for j in range(NGRP[c]):
                    a = cc * CK + CK - 16 * (j + 1)
                    rows.append(kk[a:a + 16, :])
            ko = jnp.concatenate(rows, axis=0).astype(bf16).astype(f32)
            g0 = GBASE[r * CPR]
            n = len(rows)
            for h in range(H):
                j = h // 6
                lo = DH * h - SLAB_OFF[j]
                blk = ko[:, j * 128:(j + 1) * 128]
                if lo:
                    blk = pltpu.roll(blk, 128 - lo, axis=1)
                koff_s[h, g0 * 16:(g0 + n) * 16, :] = blk
        return kmax

    def qproj(r, kcol):
        xn = xn_s[pl.ds(r * RC, RC), :]
        qt = jax.lax.dot_general(wqvt_s[0:D, :], xn, (((1,), (1,)), ((), ())),
                                 preferred_element_type=f32) * (DH ** -0.5 * LOG2E)
        qn2 = jnp.dot(ind_q(), (qt * qt).astype(bf16), preferred_element_type=f32)
        nb = SHIFT - jnp.sqrt(qn2 * jnp.concatenate([kcol] * (RC // 128), axis=1)) * 1.02
        nb = nb.astype(bf16).astype(f32)
        qr = qt.astype(bf16).astype(f32)
        row32 = jax.lax.broadcasted_iota(i32, (32, RC), 0)
        row16 = jax.lax.broadcasted_iota(i32, (16, RC), 0)
        row24 = jax.lax.broadcasted_iota(i32, (24, RC), 0)
        for h in range(H):
            js = h // 6
            off = SLAB_OFF[js]
            lo = DH * h - off
            t = lo // 16
            l2 = lo - 16 * t
            nbh = nb[h:h + 1, :]
            blk = jnp.where((row32 >= l2) & (row32 < l2 + DH), qr[off + 16 * t:off + 16 * t + 32, :], 0.0)
            ot = ONES_LANE[js] // 16
            orow = ONES_LANE[js] % 16
            if t <= ot <= t + 1:
                blk = jnp.where(row32 == (ot - t) * 16 + orow, nbh, blk)
            else:
                qm_s[r * H + h, 8 * ot:8 * ot + 8, :] = pltpu.bitcast(
                    jnp.where(row16 == orow, nbh, 0.0).astype(bf16), u32)
            qm_s[r * H + h, 8 * t:8 * t + 16, :] = pltpu.bitcast(blk.astype(bf16), u32)
            if NB:
                base = (DH * h // 8) * 8
                brow = 20 if h % 2 == 0 else 0
                qw_s[r * H + h] = jnp.where(row24 == brow, nbh, qr[base:base + 24, :])

    def vproj(r):
        xn = xn_s[pl.ds(r * RC, RC), :]
        vt = jax.lax.dot_general(wqvt_s[D:2 * D, :], xn, (((1,), (1,)), ((), ())),
                                 preferred_element_type=f32)
        vt = vt.astype(bf16).astype(f32)
        row24 = jax.lax.broadcasted_iota(jnp.int32, (24, RC), 0)
        for h in range(H):
            base = (DH * h // 8) * 8
            ones_row = 20 if h % 2 == 0 else 0
            vt_s[r, h] = jnp.where(row24 == ones_row, 1.0, vt[base:base + 24, :])

    state = dict(h=0, cnt=0, neg=0)

    def gate(val, tok):
        mask = jax.lax.broadcasted_iota(i32, (8, 128), 1) < state['neg']
        return jnp.where(mask, tok, val)

    def build_kb(h, par, d, gs, z):
        for g in gs:
            for half in range(2):
                ko = koff_s[h, pl.ds(g * 16 + half * 8, 8), :]
                if z is not None:
                    ko = gate(ko, z)
                kbuf[par][g, d, half * 8:half * 8 + 8, :] = jnp.broadcast_to(ko[:, d:d + 1], (8, 128))

    def zfill(i, carry):
        qm_s[i] = jnp.zeros((64, TQ), u32)
        return carry
    jax.lax.fori_loop(0, 3 * H + 16, zfill, 0)
    cp_x0.wait()
    qm_s[3 * H + 16:4 * H] = jnp.zeros((H - 16, 64, TQ), u32)
    zero_s[...] = jnp.zeros(zero_s.shape, f32)
    acc_s[...] = jnp.zeros(acc_s.shape, f32)
    for pb in pbufs:
        pb[...] = jnp.zeros(pb.shape, u32)
    ln(0)
    cp_wk.wait()
    for j in range(NSLAB):
        wk_s[:, j * 128:(j + 1) * 128] = wkr_s[:, SLAB_OFF[j]: SLAB_OFF[j] + 128]
    kmax = kproj(0, None)
    cp_xr.wait()
    cp_wq.wait()
    cp_wv.wait()
    for c in late:
        c.start()
    ln(1)
    kmax = kproj(1, kmax)
    wqvt_s[D:2 * D, :] = wv_s[...].T
    ln(2)
    kmax = kproj(2, kmax)
    wqvt_s[0:D, :] = wq_s[...].T
    ln(3)
    kmax = kproj(3, kmax)
    krow = jnp.max(kmax, axis=0, keepdims=True)
    kcol = jnp.broadcast_to(krow, (128, 128)).T[0:H, :]
    vproj(0)
    qproj(0, kcol)
    for d in range(DH):
        build_kb(0, 0, d, range(NB), None)
    for r in range(1, NR):
        vproj(r)
        qproj(r, kcol)

    def vpu_block(h, par, gb, z):
        qt, i = divmod(gb, BPI)
        c, j, t0 = BLIST[i]
        u = qt * NCK + c
        state['cnt'] += 1
        z0 = (state['h'] + state['cnt']) >> 20
        qi = qt * H + h + z0
        row = lambda d: d if par == 0 else (d + 4) % 24
        accs = []
        for t in range(t0, t0 + NT):
            accs.append(jnp.broadcast_to(qw_s[qi, row(DH):row(DH) + 1, t * 128:(t + 1) * 128], (16, 128)))
        for d in range(DH):
            kb = kbuf[par][GBASE[c] + j + z0, d]
            for ti, t in enumerate(range(t0, t0 + NT)):
                qb = qw_s[qi, row(d):row(d) + 1, t * 128:(t + 1) * 128]
                if d == GATE:
                    qb = gate(jnp.broadcast_to(qb, (8, 128)), z)
                    qb = jnp.concatenate([qb, qb], axis=0)
                accs[ti] = accs[ti] + kb * qb
        acc = jnp.concatenate(accs, axis=1)
        p = pltpu.bitcast(jnp.exp2(acc).astype(bf16), u32)
        r0 = (CK - 16 * (j + 1)) // 2
        pbufs[u % NPB][pl.ds(r0, 8), pl.ds(t0 * 128, NT * 128)] = p

    def qk_unit(h, u):
        qt, c = divmod(u, NCK)
        nm = CK - 16 * NGRP[c]
        kc = pltpu.bitcast(k_s[h // 6, pl.ds(c * (CK // 2), nm // 2), :], bf16)
        s = jnp.dot(kc, pltpu.bitcast(qm_s[qt * H + h], bf16), preferred_element_type=f32)
        pbufs[u % NPB][pl.ds(0, nm // 2), :] = pltpu.bitcast(jnp.exp2(s).astype(bf16), u32)
        zs = []
        for ti in range(NTOK):
            r = ((ti * nm) // NTOK) // 8 * 8
            zs.append(s[r:r + 8, 0:128])
        return zs

    def pv_unit(h, u, acc, zp):
        kc = (u % NCK) * CK
        p = pltpu.bitcast(pbufs[u % NPB][pl.ds(zp, 64), :], bf16)
        o = jnp.dot(vt_s[kc // RC, h, :, pl.ds(kc % RC, CK)], p, preferred_element_type=f32)
        return acc + o

    span = (0, UPH - 2)

    def block(h, par):
        state['h'] = h
        state['neg'] = h >> 20
        zp = pl.multiple_of((h >> 20) * 8, 8)
        hp = jnp.maximum(h - 1, 0)
        hn = jnp.minimum(h + 1, H - 1)
        acc = acc_s[...]
        for v in range(UPH):
            u = v - LEAD
            zs = qk_unit(h if u >= 0 else hp, u % UPH)
            for ti in range(NTOK):
                if ti % (NTOK // NBAT) == 0 and span[0] <= v < span[1]:
                    n = (span[1] - span[0]) * NBAT
                    tot = DH * NB
                    k = (v - span[0]) * NBAT + ti // (NTOK // NBAT)
                    idxs = range((k * tot) // n, ((k + 1) * tot) // n)
                    for d in sorted(set(i // NB for i in idxs)):
                        build_kb(hn, 1 - par, d, [i % NB for i in idxs if i // NB == d], zs[ti])
                a = v * NTOK + ti
                for gb in range((a * BPI) // TPI, ((a + 1) * BPI) // TPI):
                    vpu_block(h, par, gb, zs[ti])
            w = u - LAGU
            hw = h if w >= 0 else hp
            qt, c = divmod(w % UPH, NCK)
            if c == 0:
                acc = zero_s[h >> 20]
            acc = pv_unit(hw, w % UPH, acc, zp)
            if c == NCK - 1:
                oraw_s[hw * NQ + qt] = acc
        acc_s[...] = acc

    def body(b, carry):
        pl.when((b >> 20) == 0)(lambda: block(2 * b, 0))
        pl.when((b >> 21) == 0)(lambda: block(2 * b + 1, 1))
        return carry

    jax.lax.fori_loop(0, H // 2, body, 0)

    for u in range(UPH - LEAD, UPH):
        qk_unit(H - 1, u)
    acc = acc_s[...]
    for w in range(UPH - LEAD - LAGU, UPH):
        acc = pv_unit(H - 1, w, acc, 0)
    oraw_s[H * NQ - 1] = acc

    def chk(g, carry):
        lo, hi = carry
        for par in range(2):
            for qt in range(NQ):
                a = oraw_s[(2 * g + par) * NQ + qt]
                lrow = 20 if par == 0 else 0
                lo = jnp.minimum(lo, a[lrow:lrow + 1, :])
                aa = jnp.abs(a)
                big = jnp.maximum(jnp.maximum(aa[0:8], aa[8:16]), aa[16:24])
                hi = jnp.maximum(hi, jnp.where(big <= L_MAX, 0.0, 1.0))
        return lo, hi
    lo, hi = jax.lax.fori_loop(0, H // 2, chk, (jnp.full((1, TQ), 1.0, f32), jnp.zeros((8, TQ), f32)))
    bad = jnp.max(jnp.where(lo >= L_MIN, 0.0, 1.0)) + jnp.max(hi)
    if FORCE_FB:
        bad = bad + 1.0

    @pl.when(bad > 0.0)
    def _fallback():
        def item(it, carry):
            h = it // NQ
            qt = it % NQ
            w = pltpu.bitcast(qm_s[qt * H + h], bf16)

            def p1(c, m):
                kc = pltpu.bitcast(k_s[h // 6, pl.ds(pl.multiple_of(c * (CK // 2), CK // 2), CK // 2), :], bf16)
                s = jnp.dot(kc, w, preferred_element_type=f32)
                sfb_s[pl.ds(pl.multiple_of(c * CK, CK), CK), :] = s
                return jnp.maximum(m, jnp.max(s.reshape(CK // 8, 8, TQ), axis=0))
            m = jax.lax.fori_loop(0, NCK, p1, jnp.full((8, TQ), -jnp.inf, f32))
            m = jnp.max(m, axis=0, keepdims=True)

            def p2(r, acc):
                s = sfb_s[pl.ds(pl.multiple_of(r * RC, RC), RC), :]
                p = jnp.exp2(s - m).astype(bf16)
                return acc + jnp.dot(vt_s[r, h], p, preferred_element_type=f32)
            oraw_s[it] = jax.lax.fori_loop(0, NR, p2, jnp.zeros((24, TQ), f32))
            return carry
        jax.lax.fori_loop(0, H * NQ, item, 0)

    for c in late:
        c.wait()

    def out_copy(t):
        return pltpu.make_async_copy(out_s.at[pl.ds(t * TT, TT), :], o_hbm.at[pl.ds(t * TT, TT), :], sem_out.at[t])

    def tail_tile(qt, i):
        t = qt * (TQ // TT) + i
        rows = pl.ds(pl.multiple_of(t * TT, TT), TT)
        xn = xn_s[rows, :]
        acc = x_s[rows, :].astype(f32)
        for fc in range(F // FC):
            cols = slice(fc * FC, (fc + 1) * FC)
            g = jnp.dot(xn, wg_s[:, cols], preferred_element_type=f32)
            u = jnp.dot(xn, wu_s[:, cols], preferred_element_type=f32)
            hh = (g * jax.nn.sigmoid(g) * u).astype(bf16)
            acc = acc + jnp.dot(hh, wd_s[cols, :], preferred_element_type=f32)
        row8 = jax.lax.broadcasted_iota(jnp.int32, (8, TT), 0)
        lanes = pl.ds(pl.multiple_of(i * TT, TT), TT)
        pieces = []
        for g in range(H // 2):
            a = oraw_s[2 * g * NQ + qt, :, lanes]
            b = oraw_s[(2 * g + 1) * NQ + qt, :, lanes]
            a = a * (1.0 / a[20:21, :])
            b = b * (1.0 / b[0:1, :])
            pieces += [a[0:16], jnp.where(row8 < 4, a[16:24], b[0:8]), b[8:24]]
        ot = jnp.concatenate(pieces, axis=0).astype(bf16)
        acc = acc + jax.lax.dot_general(ot, wo_s[...], (((0,), (0,)), ((), ())),
                                        preferred_element_type=f32)
        out_s[rows, :] = acc.astype(bf16)
        pltpu.make_async_copy(out_s.at[rows, :], o_hbm.at[rows, :], sem_out.at[t]).start()

    def tail(t, carry):
        tail_tile(t // (TQ // TT), t % (TQ // TT))
        return carry

    jax.lax.fori_loop(0, S // TT, tail, 0)
    for t in range(S // TT):
        out_copy(t).wait()


@jax.jit
def pallas_parallel_sum__mha_block__swiglu_ffn__prompt_kernel(A_x, A_wqkv, A_wo, B_x, B_w_gate, B_w_up, B_w_down):
    x = A_x.reshape(S, D)
    bf16 = jnp.bfloat16
    f32 = jnp.float32
    u32 = jnp.uint32
    nb = max(NB, 1)
    anyspec = pl.BlockSpec(memory_space=pl.ANY)
    out = pl.pallas_call(
        _kernel,
        in_specs=[anyspec] * 6,
        out_specs=anyspec,
        out_shape=jax.ShapeDtypeStruct((S, D), bf16),
        scratch_shapes=[
            pltpu.VMEM((S, D), bf16),
            pltpu.VMEM((D, D), bf16),
            pltpu.VMEM((D, D), bf16),
            pltpu.VMEM((D, D), bf16),
            pltpu.VMEM((D, D), bf16),
            pltpu.VMEM((D, F), bf16),
            pltpu.VMEM((D, F), bf16),
            pltpu.VMEM((F, D), bf16),
            pltpu.VMEM((S, D), bf16),
            pltpu.VMEM((S, D), bf16),
            pltpu.VMEM((D, NSLAB * 128), bf16),
            pltpu.VMEM((2 * D, D), bf16),
            pltpu.VMEM((NSLAB, S // 2, 128), u32),
            pltpu.VMEM((NQ * H, 64, TQ), u32),
            pltpu.VMEM((S // RC, H, 24, RC), f32),
            pltpu.VMEM((H * NQ, 24, TQ), f32),
            pltpu.VMEM((H, nb * 16, 128), f32),
            pltpu.VMEM((NQ * H, 24, TQ), f32),
            pltpu.VMEM((nb, DH, 16, 128), f32),
            pltpu.VMEM((nb, DH, 16, 128), f32),
            pltpu.VMEM((1, 24, TQ), f32),
            pltpu.VMEM((24, TQ), f32),
            pltpu.VMEM((S, TQ), f32),
        ] + [pltpu.VMEM((64, TQ), u32)] * NPB + [
            pltpu.SemaphoreType.DMA((9,)),
            pltpu.SemaphoreType.DMA((S // TT,)),
        ],
        compiler_params=pltpu.CompilerParams(
            vmem_limit_bytes=110 * 1024 * 1024),
        name="fused_block",
    )(x, A_wqkv, A_wo, B_w_gate, B_w_up, B_w_down)
    return out.reshape(1, S, D)
```

```python
import bisect
import os

import jax
import jax.numpy as jnp
import jax.experimental.pallas as pl
import jax.experimental.pallas.tpu as pltpu

S = 2048
D = 640
H = 32
DH = 20
F = 1536
EPS = 1e-5
NSLAB = 6
SLAB_OFF = (0, 120, 240, 360, 480, 512)
ONES_LANE = (127, 127, 127, 127, 127, 0)
LOG2E = 1.4426950408889634
SHIFT = 100.0
L_MIN = 2.0 ** -80
L_MAX = 2.0 ** 124

TQ = 512
CK = 128
NCK = S // CK
NQ = S // TQ
RC = 512
NR = S // RC
CPR = RC // CK
_e = lambda k, d: int(os.environ.get(k, d))
TT = _e('TT', 512)
NB = _e('NB', 20)
NTOK = 8
GATE = 19
LAGU = 2
LEAD = 1
NPB = 8
KB3 = _e('KB3', 2)
PH = 0.5
FM = S // H
FT = 4
FORCE_FB = _e('FORCE_FB', 0)

NGRP = [((c + 1) * NB) // NCK - (c * NB) // NCK for c in range(NCK)]
GBASE = [(c * NB) // NCK for c in range(NCK)]
UPH = NQ * NCK
BLIST = [(qt, c, j, t) for qt in range(NQ) for c in range(NCK) for j in range(NGRP[c]) for t in range(4)]


def _plan():
    pieces = [('gu', j) for j in range(6)] + [('dn', n) for n in range(5)]
    nsub = {'gu': 5, 'dn': 3}
    ppos = {1 + (i * (UPH - 3)) // len(pieces): p for i, p in enumerate(pieces)}
    ttime, tunit, tok0 = [], [], {}
    t = 0
    for v in range(UPH):
        nm = CK - 16 * NGRP[(v - LEAD) % NCK]
        tok0[(v, 'qk')] = len(ttime)
        for ti in range(NTOK):
            ttime.append(t + (ti * nm) // NTOK)
            tunit.append(v)
        t += nm + 24
        if v in ppos:
            tok0[(v, 'ffn')] = len(ttime)
            for _ in range(nsub[ppos[v][0]]):
                for ti in range(FT):
                    ttime.append(t + ti * (FM // FT))
                    tunit.append(v + 1)
                t += FM
    assign = [[] for _ in ttime]
    kassign = [[] for _ in ttime]
    for i, (qt, c, j, _) in enumerate(BLIST):
        k = min(bisect.bisect_left(ttime, (i + PH) * t / len(BLIST)), len(ttime) - 1)
        assign[k].append(i)
        u = qt * NCK + c
        assert u - (NPB - LAGU - LEAD - 1) <= tunit[k] <= u + LEAD + LAGU - 1
    nk = DH * NB
    for i in range(nk):
        kassign[bisect.bisect_left(ttime, (i // KB3 * KB3) * ttime[-2 * NTOK] / nk)].append(i)
    return ppos, nsub, tok0, assign, kassign


PPOS, NSUB, TOK0, ASSIGN, KASSIGN = _plan()


def _kernel(x_hbm, wqkv_hbm, wo_hbm, wg_hbm, wu_hbm, wd_hbm, o_hbm,
            x_s, wq_s, wkr_s, wv_s, wo_s, wg_s, wu_s, wd_s, out_s,
            xn_s, wk_s, wqvt_s, k_s, qm_s, vt_s, oraw_s, koff_s, qw_s, kb_a, kb_b,
            wgu_p, wd_p, hh_s, y_s, zero_s, acc_s, kcol_s, vmax_s, rinv_s, flag_s, sfb_s,
            p0, p1, p2, p3, p4, p5, p6, p7, sem_in, sem_out):
    f32 = jnp.float32
    bf16 = jnp.bfloat16
    u32 = jnp.uint32
    i32 = jnp.int32
    pbufs = (p0, p1, p2, p3, p4, p5, p6, p7)
    kbuf = (kb_a, kb_b)

    cp_x0 = pltpu.make_async_copy(x_hbm.at[pl.ds(0, RC), :], x_s.at[pl.ds(0, RC), :], sem_in.at[0])
    cp_wk = pltpu.make_async_copy(wqkv_hbm.at[:, pl.ds(D, D)], wkr_s, sem_in.at[1])
    cp_wq = pltpu.make_async_copy(wqkv_hbm.at[:, pl.ds(0, D)], wq_s, sem_in.at[2])
    cp_wv = pltpu.make_async_copy(wqkv_hbm.at[:, pl.ds(2 * D, D)], wv_s, sem_in.at[3])
    cp_x1 = pltpu.make_async_copy(x_hbm.at[pl.ds(RC, RC), :], x_s.at[pl.ds(RC, RC), :], sem_in.at[4])
    cp_xr = pltpu.make_async_copy(x_hbm.at[pl.ds(2 * RC, 2 * RC), :], x_s.at[pl.ds(2 * RC, 2 * RC), :], sem_in.at[9])
    late = [pltpu.make_async_copy(src, dst, sem_in.at[5 + i])
            for i, (src, dst) in enumerate(((wg_hbm, wg_s), (wu_hbm, wu_s), (wd_hbm, wd_s), (wo_hbm, wo_s)))]
    cp_x0.start()
    cp_wk.start()
    cp_wv.start()
    cp_x1.start()
    cp_xr.start()
    cp_wq.start()
    flag_s[0] = 0
    flag_s[1] = 0

    state = dict(h=0, cnt=0, neg=0)

    def gate(val, tok):
        mask = jax.lax.broadcasted_iota(i32, (8, 128), 1) < state['neg']
        return jnp.where(mask, tok, val)

    def xn_chunk(r):
        start = r * (RC // 2)
        if not isinstance(r, int):
            start = pl.multiple_of(start, RC // 2)
        return pltpu.bitcast(xn_s[pl.ds(start, RC // 2), :], bf16)

    def ln(r):
        x = x_s[pl.ds(r * RC, RC), :].astype(f32)
        mu = jnp.mean(x, axis=-1, keepdims=True)
        xc = x - mu
        var = jnp.mean(xc * xc, axis=-1, keepdims=True)
        xn_s[pl.ds(r * (RC // 2), RC // 2), :] = pltpu.bitcast((xc * jax.lax.rsqrt(var + EPS)).astype(bf16), u32)

    def ind_k():
        l = jax.lax.broadcasted_iota(i32, (NSLAB * 128, 128), 0)
        h = jax.lax.broadcasted_iota(i32, (NSLAB * 128, 128), 1)
        j = jnp.minimum(h // 6, 5)
        start = j * 128 + DH * h - jnp.where(j < 5, 120 * j, SLAB_OFF[5])
        return jnp.where((l >= start) & (l < start + DH) & (h < H), 1.0, 0.0).astype(bf16)

    def kproj(r, kmax):
        kk = jnp.dot(xn_chunk(r), wk_s[...], preferred_element_type=f32)
        k2 = kk * kk
        k2 = jnp.maximum(k2[0:RC // 2], k2[RC // 2:RC]).astype(bf16)
        kn2 = jnp.dot(k2, ind_k(), preferred_element_type=f32)
        kn2 = jnp.max(kn2.reshape(RC // 16, 8, 128), axis=0)
        kmax = kn2 if kmax is None else jnp.maximum(kmax, kn2)
        for h in range(H):
            js = h // 6
            t = (DH * h - SLAB_OFF[js]) // 16
            ot = ONES_LANE[js] // 16
            tr = (h % 8) * 64
            tc = (h // 8 + 2 if h >= 16 else h // 8) * 128
            zt = pltpu.bitcast(gate(jnp.zeros((8, 128), f32), kk[tr:tr + 8, tc:tc + 128]), u32)
            zt = jnp.concatenate([zt] * (TQ // 128), axis=1)
            for tt in range(8):
                if tt not in (t, t + 1, ot):
                    qm_s[r * H + h, 8 * tt:8 * tt + 8, :] = zt
        lane = jax.lax.broadcasted_iota(i32, (RC, 128), 1)
        for j in range(NSLAB):
            kj = jnp.where(lane == ONES_LANE[j], 1.0, kk[:, j * 128:(j + 1) * 128]).astype(bf16)
            k_s[j, pl.ds(r * (RC // 2), RC // 2), :] = pltpu.bitcast(kj, u32)
        rows = []
        for cc in range(CPR):
            c = r * CPR + cc
            for j in range(NGRP[c]):
                a = cc * CK + CK - 16 * (j + 1)
                rows.append(kk[a:a + 16, :])
        ko = jnp.concatenate(rows, axis=0).astype(bf16).astype(f32)
        g0 = GBASE[r * CPR]
        n = len(rows)
        for h in range(H):
            j = h // 6
            lo = DH * h - SLAB_OFF[j]
            blk = ko[:, j * 128:(j + 1) * 128]
            if lo:
                blk = pltpu.roll(blk, 128 - lo, axis=1)
            koff_s[h, g0 * 16:(g0 + n) * 16, :] = blk
        return kmax

    HG = 8
    MG = HG * DH

    def qproj(r, side=None):
        xn = xn_chunk(r)
        row32 = jax.lax.broadcasted_iota(i32, (32, RC), 0)
        row16 = jax.lax.broadcasted_iota(i32, (16, RC), 0)
        row24 = jax.lax.broadcasted_iota(i32, (24, RC), 0)
        zpad = jnp.zeros((16, RC), f32)
        for gq in range(H // HG):
            qt = jax.lax.dot_general(wqvt_s[gq * MG:(gq + 1) * MG, :], xn, (((1,), (1,)), ((), ())),
                                     preferred_element_type=f32) * (DH ** -0.5 * LOG2E)
            if side is not None:
                side(qt)
            qr = jnp.concatenate([zpad, qt.astype(bf16).astype(f32), zpad], axis=0)
            for h in range(gq * HG, (gq + 1) * HG):
                js = h // 6
                off = SLAB_OFF[js]
                lo = DH * h - off
                t = lo // 16
                l2 = lo - 16 * t
                base = (DH * h // 8) * 8 - gq * MG + 16
                win = qr[base:base + 24, :]
                brow, v0 = (20, 0) if h % 2 == 0 else (0, 4)
                wm = jnp.where((row24 >= v0) & (row24 < v0 + DH), win, 0.0)
                qn2 = jnp.sum(wm * wm, axis=0, keepdims=True)
                kc = jnp.concatenate([kcol_s[h:h + 1, :]] * (RC // 128), axis=1)
                nbh = (SHIFT - jnp.sqrt(qn2 * kc) * 1.02).astype(bf16).astype(f32)
                qw_s[r * H + h] = jnp.where(row24 == brow, nbh, win)
                a = off + 16 * t - gq * MG + 16
                blk = jnp.where((row32 >= l2) & (row32 < l2 + DH), qr[a:a + 32, :], 0.0)
                ot = ONES_LANE[js] // 16
                orow = ONES_LANE[js] % 16
                if t <= ot <= t + 1:
                    blk = jnp.where(row32 == (ot - t) * 16 + orow, nbh, blk)
                else:
                    qm_s[r * H + h, 8 * ot:8 * ot + 8, :] = pltpu.bitcast(
                        jnp.where(row16 == orow, nbh, 0.0).astype(bf16), u32)
                qm_s[r * H + h, 8 * t:8 * t + 16, :] = pltpu.bitcast(blk.astype(bf16), u32)

    def vproj(r, wvt=None, side=None):
        xn = xn_chunk(r)
        row24 = jax.lax.broadcasted_iota(jnp.int32, (24, RC), 0)
        for gq in range(H // HG):
            w = wqvt_s[D + gq * MG:D + (gq + 1) * MG, :] if wvt is None else wvt[gq * MG:(gq + 1) * MG, :]
            vt = jax.lax.dot_general(w, xn, (((1,), (1,)), ((), ())), preferred_element_type=f32)
            if side is not None:
                side(vt)
            vt = vt.astype(bf16).astype(f32)
            vmax_s[...] = jnp.maximum(vmax_s[...], jnp.max(jnp.abs(vt).reshape(MG // 8, 8, RC), axis=0))
            for h in range(gq * HG, (gq + 1) * HG):
                base = (DH * h // 8) * 8 - gq * MG
                ones_row = 20 if h % 2 == 0 else 0
                vt_s[r, h] = jnp.where(row24 == ones_row, 1.0, vt[base:base + 24, :])

    def build_kb(h, par, d, gs, z):
        for g in gs:
            for half in range(2):
                st = g * 16 + half * 8
                ko = koff_s[h, pl.ds(st if isinstance(st, int) else pl.multiple_of(st, 8), 8), :]
                if z is not None:
                    ko = gate(ko, z)
                kbuf[par][g, d, half * 8:half * 8 + 8, :] = jnp.broadcast_to(ko[:, d:d + 1], (8, 128))

    state['neg'] = flag_s[1]
    zero_s[...] = jnp.zeros(zero_s.shape, f32)
    acc_s[...] = jnp.zeros(acc_s.shape, f32)
    vmax_s[...] = jnp.zeros(vmax_s.shape, f32)
    for pb in pbufs:
        pb[...] = jnp.zeros(pb.shape, u32)
    cp_x0.wait()
    ln(0)
    cp_wk.wait()
    for j in range(NSLAB):
        wk_s[:, j * 128:(j + 1) * 128] = wkr_s[:, SLAB_OFF[j]: SLAB_OFF[j] + 128]
    kmax = kproj(0, None)
    cp_wv.wait()
    cp_x1.wait()
    for c in late:
        c.start()
    wvt = wv_s[...].T
    wqvt_s[D:2 * D, :] = wvt
    vproj(0, wvt)
    ln(1)
    kmax = kproj(1, kmax)
    cp_xr.wait()
    cp_wq.wait()
    vproj(1)
    ln(2)
    kmax = kproj(2, kmax)
    wqvt_s[0:D, :] = wq_s[...].T
    ln(3)
    kmax = kproj(3, kmax)
    krow = jnp.max(kmax, axis=0, keepdims=True)
    kcol_s[...] = jnp.broadcast_to(krow, (128, 128)).T[0:H, :]
    for c in late:
        c.wait()

    def gate_u32(val, tok):
        r, c = val.shape
        mask = jax.lax.broadcasted_iota(i32, (r, c), 1) < state['neg']
        t = pltpu.bitcast(tok, u32)
        t = jnp.concatenate([jnp.concatenate([t] * (c // 128), axis=1)] * (r // 8), axis=0)
        return jnp.where(mask, t, val)

    def qvloop(i, carry):
        jobs = []
        kr = pl.ds(pl.multiple_of(i * (D // 2), D // 2), D // 2)
        kr2 = pl.ds(pl.multiple_of(i * (D // 4), D // 4), D // 4)
        fr = pl.ds(pl.multiple_of(i * (F // 2), F // 2), F // 2)
        fr2 = pl.ds(pl.multiple_of(i * (F // 4), F // 4), F // 4)
        for j in range(12):
            def job_g(tok, j=j):
                o = (j % 2) * 128
                wgu_p[j // 2, kr2, o:o + 128] = gate_u32(pltpu.bitcast(wg_s[kr, j * 128:(j + 1) * 128], u32), tok)
            def job_u(tok, j=j):
                o = 256 + (j % 2) * 128
                wgu_p[j // 2, kr2, o:o + 128] = gate_u32(pltpu.bitcast(wu_s[kr, j * 128:(j + 1) * 128], u32), tok)
            jobs += [job_g, job_u]
        for n in range(5):
            def job_d(tok, n=n):
                wd_p[n, fr2, :] = gate_u32(pltpu.bitcast(wd_s[fr, n * 128:(n + 1) * 128], u32), tok)
            jobs.append(job_d)
        for d in range(DH):
            def job_k(tok, d=d):
                build_kb(0, 0, d, [i * (NB // 2) + g for g in range(NB // 2)], tok)
            jobs.insert(2 * d + 1, job_k)
        nside = 11
        cnt = [0]

        def side(res):
            k = cnt[0]
            cnt[0] += 1
            mine = jobs[(k * len(jobs)) // nside:((k + 1) * len(jobs)) // nside] if k < nside else []
            for n, job in enumerate(mine):
                rr = (n * MG // len(mine)) // 8 * 8
                job(res[rr:rr + 8, 0:128])

        qproj(2 * i, side)
        qproj(2 * i + 1, side)
        vproj(2 + i, None, side)
        return carry

    jax.lax.fori_loop(0, 2, qvloop, 0)

    def opaque_zero():
        state['cnt'] += 1
        return (state['h'] + state['cnt']) >> 20

    def vpu_block(h, par, i, z):
        qt, c, j, t = BLIST[i]
        u = qt * NCK + c
        z0 = opaque_zero()
        qi = qt * H + h + z0
        row = lambda d: d if par == 0 else (d + 4) % 24
        lanes = slice(t * 128, (t + 1) * 128)
        acc = jnp.broadcast_to(qw_s[qi, row(DH):row(DH) + 1, lanes], (16, 128))
        for d in range(DH):
            kb = kbuf[par][GBASE[c] + j + z0, d]
            qb = qw_s[qi, row(d):row(d) + 1, lanes]
            if d == GATE:
                qb = gate(jnp.broadcast_to(qb, (8, 128)), z)
                qb = jnp.concatenate([qb, qb], axis=0)
            acc = acc + kb * qb
        r0 = (CK - 16 * (j + 1)) // 2
        pbufs[u % NPB][r0:r0 + 8, lanes] = pltpu.bitcast(jnp.exp2(acc).astype(bf16), u32)

    def qk_unit(h, u):
        qt, c = divmod(u, NCK)
        nm = CK - 16 * NGRP[c]
        kc = pltpu.bitcast(k_s[h // 6, pl.ds(c * (CK // 2), nm // 2), :], bf16)
        s = jnp.dot(kc, pltpu.bitcast(qm_s[qt * H + h], bf16), preferred_element_type=f32)
        pbufs[u % NPB][pl.ds(0, nm // 2), :] = pltpu.bitcast(jnp.exp2(s).astype(bf16), u32)
        zs = []
        for ti in range(NTOK):
            r = ((ti * nm) // NTOK) // 8 * 8
            zs.append(s[r:r + 8, 0:128])
        return zs

    def pv_unit(h, u, acc, zp):
        kc = (u % NCK) * CK
        p = pltpu.bitcast(pbufs[u % NPB][pl.ds(zp, 64), :], bf16)
        o = jnp.dot(vt_s[kc // RC, h, :, pl.ds(kc % RC, CK)], p, preferred_element_type=f32)
        return acc + o

    def ffn_piece(h, p, side):
        kind, j = p
        z0 = opaque_zero()
        acc = None
        for sidx in range(NSUB[kind]):
            if kind == 'gu':
                rows = pl.ds(pl.multiple_of((h + z0) * (FM // 2), FM // 2), FM // 2)
                a = pltpu.bitcast(xn_s[rows, sidx * 128:(sidx + 1) * 128], bf16)
                w = pltpu.bitcast(wgu_p[j, sidx * 64:(sidx + 1) * 64, :], bf16)
            else:
                a = pltpu.bitcast(hh_s[pl.ds(pl.multiple_of(z0 * 8, 8), FM // 2), sidx * 512:(sidx + 1) * 512], bf16)
                w = pltpu.bitcast(wd_p[j, sidx * 256:(sidx + 1) * 256, :], bf16)
            o = jnp.dot(a, w, preferred_element_type=f32)
            acc = o if acc is None else acc + o
            side(sidx * FT, [o[ti * (FM // FT):ti * (FM // FT) + 8, 0:128] for ti in range(FT)])
        if kind == 'gu':
            g = acc[:, :256]
            u = acc[:, 256:]
            hh = (g * u) * (0.5 * jnp.tanh(0.5 * g) + 0.5)
            hh_s[:, j * 256:(j + 1) * 256] = pltpu.bitcast(hh.astype(bf16), u32)
        else:
            y_s[pl.ds(pl.multiple_of(h * FM, FM), FM), j * 128:(j + 1) * 128] = acc

    def block(h, par):
        state['h'] = h
        state['neg'] = h >> 20
        zp = pl.multiple_of((h >> 20) * 8, 8)
        hp = jnp.maximum(h - 1, 0)
        hn = jnp.minimum(h + 1, H - 1)
        acc = acc_s[...]

        def side(k0, zs):
            for ti, z in enumerate(zs):
                idxs = KASSIGN[k0 + ti]
                for d in sorted(set(i // NB for i in idxs)):
                    build_kb(hn, 1 - par, d, [i % NB for i in idxs if i // NB == d], z)
                for i in ASSIGN[k0 + ti]:
                    vpu_block(h, par, i, z)

        for v in range(UPH):
            u = v - LEAD
            side(TOK0[(v, 'qk')], qk_unit(h if u >= 0 else hp, u % UPH))
            w = u - LAGU
            hw = h if w >= 0 else hp
            qt, c = divmod(w % UPH, NCK)
            if c == 0:
                acc = zero_s[h >> 20]
            acc = pv_unit(hw, w % UPH, acc, zp)
            if c == NCK - 1:
                oraw_s[hw * NQ + qt] = acc
            if v in PPOS:
                ffn_piece(h, PPOS[v], lambda o, zs: side(TOK0[(v, 'ffn')] + o, zs))
        acc_s[...] = acc

    def body(b, carry):
        pl.when((b >> 20) == 0)(lambda: block(2 * b, 0))
        pl.when((b >> 21) == 0)(lambda: block(2 * b + 1, 1))
        return carry

    jax.lax.fori_loop(0, H // 2, body, 0)

    for u in range(UPH - LEAD, UPH):
        qk_unit(H - 1, u)
    acc = acc_s[...]
    for w in range(UPH - LEAD - LAGU, UPH):
        acc = pv_unit(H - 1, w, acc, 0)
    oraw_s[H * NQ - 1] = acc

    def fallback():
        def item(it, carry):
            h = it // NQ
            qt = it % NQ
            w = pltpu.bitcast(qm_s[qt * H + h], bf16)

            def p1(c, m):
                kc = pltpu.bitcast(k_s[h // 6, pl.ds(pl.multiple_of(c * (CK // 2), CK // 2), CK // 2), :], bf16)
                s = jnp.dot(kc, w, preferred_element_type=f32)
                sfb_s[pl.ds(pl.multiple_of(c * CK, CK), CK), :] = s
                return jnp.maximum(m, jnp.max(s.reshape(CK // 8, 8, TQ), axis=0))
            m = jax.lax.fori_loop(0, NCK, p1, jnp.full((8, TQ), -jnp.inf, f32))
            m = jnp.max(m, axis=0, keepdims=True)

            def p2(r, acc):
                s = sfb_s[pl.ds(pl.multiple_of(r * RC, RC), RC), :]
                p = jnp.exp2(s - m).astype(bf16)
                return acc + jnp.dot(vt_s[r, h], p, preferred_element_type=f32)
            oraw_s[it] = jax.lax.fori_loop(0, NR, p2, jnp.zeros((24, TQ), f32))
            return carry
        jax.lax.fori_loop(0, H * NQ, item, 0)

    def out_copy(t):
        return pltpu.make_async_copy(out_s.at[pl.ds(t * TT, TT), :], o_hbm.at[pl.ds(t * TT, TT), :], sem_out.at[t])

    def tail(t, carry):
        lo, hi = carry
        qt = t // (TQ // TT)
        i = t % (TQ // TT)
        rows = pl.ds(pl.multiple_of(t * TT, TT), TT)
        row8 = jax.lax.broadcasted_iota(jnp.int32, (8, TT), 0)
        lanes = pl.ds(pl.multiple_of(i * TT, TT), TT)
        pieces = []
        for g8 in range(H // 8):
            lst = None
            for k in range(8):
                h = g8 * 8 + k
                lrow = 20 if h % 2 == 0 else 0
                lk = jnp.concatenate(
                    [jnp.broadcast_to(oraw_s[h * NQ + qt, lrow:lrow + 1, pl.ds(pl.multiple_of(i * TT + n * 128, 128), 128)],
                                      (8, 128)) for n in range(TT // 128)], axis=1)
                lst = lk if lst is None else jnp.where(row8 == k, lk, lst)
            lo = jnp.minimum(lo, lst)
            hi = jnp.maximum(hi, lst)
            rinv_s[g8 * 8:(g8 + 1) * 8, :] = 1.0 / lst
            for g in range(g8 * 4, g8 * 4 + 4):
                ra = jnp.concatenate([jnp.broadcast_to(rinv_s[2 * g:2 * g + 1, n * 128:(n + 1) * 128], (8, 128))
                                      for n in range(TT // 128)], axis=1)
                rb = jnp.concatenate([jnp.broadcast_to(rinv_s[2 * g + 1:2 * g + 2, n * 128:(n + 1) * 128], (8, 128))
                                      for n in range(TT // 128)], axis=1)
                a = oraw_s[2 * g * NQ + qt, :, lanes]
                b = oraw_s[(2 * g + 1) * NQ + qt, :, lanes]
                pieces += [a[0:8] * ra, a[8:16] * ra,
                           jnp.where(row8 < 4, a[16:24] * ra, b[0:8] * rb), b[8:16] * rb, b[16:24] * rb]
        ot = jnp.concatenate(pieces, axis=0).astype(bf16)
        acc = x_s[rows, :].astype(f32) + y_s[rows, :]
        acc = acc + jax.lax.dot_general(ot, wo_s[...], (((0,), (0,)), ((), ())),
                                        preferred_element_type=f32)
        out_s[rows, :] = acc.astype(bf16)
        pltpu.make_async_copy(out_s.at[rows, :], o_hbm.at[rows, :], sem_out.at[t]).start()
        return lo, hi

    def one_pass(p, carry):
        @pl.when(jnp.logical_or(p == 0, flag_s[0] != 0))
        def _():
            pl.when(p == 1)(fallback)
            lo, hi = jax.lax.fori_loop(0, S // TT, tail, (jnp.ones((8, TT), f32), jnp.ones((8, TT), f32)))
            vm = jnp.maximum(jnp.max(vmax_s[...]), 1.0)
            ok = (lo >= L_MIN) & (hi * vm <= L_MAX)
            flag_s[0] = (jnp.max(jnp.where(ok, 0.0, 1.0)) > 0.0).astype(i32) + FORCE_FB
            for t in range(S // TT):
                out_copy(t).wait()
        return carry

    jax.lax.fori_loop(0, 2, one_pass, 0)


@jax.jit
def pallas_parallel_sum__mha_block__swiglu_ffn__prompt_kernel(A_x, A_wqkv, A_wo, B_x, B_w_gate, B_w_up, B_w_down):
    x = A_x.reshape(S, D)
    bf16 = jnp.bfloat16
    f32 = jnp.float32
    u32 = jnp.uint32
    anyspec = pl.BlockSpec(memory_space=pl.ANY)
    out = pl.pallas_call(
        _kernel,
        in_specs=[anyspec] * 6,
        out_specs=anyspec,
        out_shape=jax.ShapeDtypeStruct((S, D), bf16),
        scratch_shapes=[
            pltpu.VMEM((S, D), bf16),
            pltpu.VMEM((D, D), bf16),
            pltpu.VMEM((D, D), bf16),
            pltpu.VMEM((D, D), bf16),
            pltpu.VMEM((D, D), bf16),
            pltpu.VMEM((D, F), bf16),
            pltpu.VMEM((D, F), bf16),
            pltpu.VMEM((F, D), bf16),
            pltpu.VMEM((S, D), bf16),
            pltpu.VMEM((S // 2, D), u32),
            pltpu.VMEM((D, NSLAB * 128), bf16),
            pltpu.VMEM((2 * D, D), bf16),
            pltpu.VMEM((NSLAB, S // 2, 128), u32),
            pltpu.VMEM((NQ * H, 64, TQ), u32),
            pltpu.VMEM((S // RC, H, 24, RC), f32),
            pltpu.VMEM((H * NQ, 24, TQ), f32),
            pltpu.VMEM((H, NB * 16, 128), f32),
            pltpu.VMEM((NQ * H, 24, TQ), f32),
            pltpu.VMEM((NB, DH, 16, 128), f32),
            pltpu.VMEM((NB, DH, 16, 128), f32),
            pltpu.VMEM((6, D // 2, 512), u32),
            pltpu.VMEM((5, F // 2, 128), u32),
            pltpu.VMEM((FM // 2, F), u32),
            pltpu.VMEM((S, D), f32),
            pltpu.VMEM((1, 24, TQ), f32),
            pltpu.VMEM((24, TQ), f32),
            pltpu.VMEM((H, 128), f32),
            pltpu.VMEM((8, RC), f32),
            pltpu.VMEM((H, TT), f32),
            pltpu.SMEM((2,), jnp.int32),
            pltpu.VMEM((S, TQ), f32),
        ] + [pltpu.VMEM((64, TQ), u32)] * NPB + [
            pltpu.SemaphoreType.DMA((10,)),
            pltpu.SemaphoreType.DMA((S // TT,)),
        ],
        compiler_params=pltpu.CompilerParams(
            vmem_limit_bytes=116 * 1024 * 1024),
        name="fused_block",
    )(x, A_wqkv, A_wo, B_w_gate, B_w_up, B_w_down)
    return out.reshape(1, S, D)
```

```python
import bisect

import jax
import jax.numpy as jnp
import jax.experimental.pallas as pl
import jax.experimental.pallas.tpu as pltpu

S = 2048
D = 640
H = 32
DH = 20
F = 1536
EPS = 1e-5
NSLAB = 6
ONES_LANE = (127, 119, 111, 103, 95, 0)
LOG2E = 1.4426950408889634
SHIFT = 100.0
L_MIN = 2.0 ** -80
L_MAX = 2.0 ** 124

TQ = 512
CK = 128
NCK = S // CK
NQ = S // TQ
RC = 512
NR = S // RC
CPR = RC // CK
TO = 256
NB = 22
GATE = DH - 1
LAGU = 2
LEAD = 1
NPB = 8
FM = S // H
FT = 8
HG = 4

NGRP = [((c + 1) * NB) // NCK - (c * NB) // NCK for c in range(NCK)]
GBASE = [(c * NB) // NCK for c in range(NCK)]
UPH = NQ * NCK
BLIST = [(qt, c, j, t) for qt in range(NQ) for c in range(NCK) for j in range(NGRP[c]) for t in range(4)]


def _plan():
    pieces = [('gu', j) for j in range(6)] + [('dn', n) for n in range(5)]
    nsub = {'gu': 5, 'dn': 3}
    ppos = {2 + (i * (UPH - 4)) // len(pieces): p for i, p in enumerate(pieces)}
    ttime, tunit, tok0 = [], [], {}
    t = 0
    for v in range(UPH):
        nm = CK - 16 * NGRP[(v - LEAD) % NCK]
        tok0[(v, 'qk')] = len(ttime)
        for ti in range(nm // 8):
            ttime.append(t + ti * 8)
            tunit.append(v)
        t += nm
        tok0[(v, 'pv')] = len(ttime)
        for ti in range(3):
            ttime.append(t + ti * 8)
            tunit.append(v + 1)
        t += 24
        if v in ppos:
            tok0[(v, 'ffn')] = len(ttime)
            for _ in range(nsub[ppos[v][0]]):
                for ti in range(FT):
                    ttime.append(t + ti * (FM // FT))
                    tunit.append(v + 1)
                t += FM
    assign = [[] for _ in ttime]
    kassign = [[] for _ in ttime]
    for i, (qt, c, _, _) in enumerate(BLIST):
        k = min(bisect.bisect_left(ttime, (i - 1.0) * t / len(BLIST)), len(ttime) - 1)
        assign[k].append(i)
        u = qt * NCK + c
        assert u - (NPB - LAGU - LEAD - 1) <= tunit[k] <= u + LEAD + LAGU - 1
    nk = DH * NB
    for i in range(nk):
        kassign[bisect.bisect_left(ttime, i * (t - 270) / nk)].append(i)
    return ppos, nsub, tok0, assign, kassign


PPOS, NSUB, TOK0, ASSIGN, KASSIGN = _plan()


def _kernel(x_hbm, wqkv_hbm, wo_hbm, wg_hbm, wu_hbm, wd_hbm, o_hbm,
            x_s, wq_s, wk_s, wv_s, wo_s, wg_s, wu_s, wd_s, out_s,
            xn_s, wqvt_s, k_s, qm_s, vt_s, oraw_s, koff_s, qw_s, kb_a, kb_b,
            wgu_p, wd_p, hh_s, y_s, zero_s, acc_s, kcol_s, vmax_s, rinv_s, flag_s, sfb_s,
            sem_in, sem_out, *pbufs):
    f32 = jnp.float32
    bf16 = jnp.bfloat16
    u32 = jnp.uint32
    i32 = jnp.int32
    kbuf = (kb_a, kb_b)

    cp_x0 = pltpu.make_async_copy(x_hbm.at[pl.ds(0, RC), :], x_s.at[pl.ds(0, RC), :], sem_in.at[0])
    cp_wk = pltpu.make_async_copy(wqkv_hbm.at[:, pl.ds(D, D)], wk_s, sem_in.at[1])
    cp_wq = pltpu.make_async_copy(wqkv_hbm.at[:, pl.ds(0, D)], wq_s, sem_in.at[2])
    cp_wv = pltpu.make_async_copy(wqkv_hbm.at[:, pl.ds(2 * D, D)], wv_s, sem_in.at[3])
    cp_x1 = pltpu.make_async_copy(x_hbm.at[pl.ds(RC, RC), :], x_s.at[pl.ds(RC, RC), :], sem_in.at[4])
    cp_xr = pltpu.make_async_copy(x_hbm.at[pl.ds(2 * RC, 2 * RC), :], x_s.at[pl.ds(2 * RC, 2 * RC), :],
                                  sem_in.at[5])
    cp_wo = pltpu.make_async_copy(wo_hbm, wo_s, sem_in.at[6])

    def late(i):
        cps = []
        for n, (src, dst) in enumerate(((wg_hbm, wg_s), (wu_hbm, wu_s), (wd_hbm, wd_s))):
            hr = src.shape[0] // 2
            rows = pl.ds(i * hr if isinstance(i, int) else pl.multiple_of(i * hr, hr), hr)
            cps.append(pltpu.make_async_copy(src.at[rows, :], dst.at[rows, :], sem_in.at[7 + 3 * i + n]))
        return cps

    for c in (cp_x0, cp_wk, cp_wv, cp_x1, cp_xr, cp_wq):
        c.start()
    flag_s[0] = 0
    flag_s[1] = 0

    state = dict(h=0, cnt=0, neg=0)

    def gate(val, tok):
        r, c = val.shape
        mask = jax.lax.broadcasted_iota(i32, (r, c), 1) < state['neg']
        t = tok if val.dtype == tok.dtype else pltpu.bitcast(tok, val.dtype)
        t = jnp.concatenate([jnp.concatenate([t] * (c // 128), axis=1)] * (r // 8), axis=0)
        return jnp.where(mask, t, val)

    def xn_chunk(r):
        start = r * (RC // 2)
        if not isinstance(r, int):
            start = pl.multiple_of(start, RC // 2)
        return pltpu.bitcast(xn_s[pl.ds(start, RC // 2), :], bf16)

    def ln(r):
        x = x_s[pl.ds(r * RC, RC), :].astype(f32)
        mu = jnp.mean(x, axis=-1, keepdims=True)
        xc = x - mu
        var = jnp.mean(xc * xc, axis=-1, keepdims=True)
        xn_s[pl.ds(r * (RC // 2), RC // 2), :] = pltpu.bitcast((xc * jax.lax.rsqrt(var + EPS)).astype(bf16), u32)

    def ind_k():
        l = jax.lax.broadcasted_iota(i32, (D, 128), 0)
        h = jax.lax.broadcasted_iota(i32, (D, 128), 1)
        return jnp.where((l >= DH * h) & (l < DH * h + DH), 1.0, 0.0).astype(bf16)

    def q_tiles(h):
        t0 = (DH * h) // 16
        return t0, (t0 % 8, (t0 + 1) % 8), ONES_LANE[h // 6] // 16

    def kproj(r, kmax):
        kk = jnp.dot(xn_chunk(r), wk_s[...], preferred_element_type=f32)
        k2 = kk * kk
        k2 = jnp.maximum(k2[0:RC // 2], k2[RC // 2:RC]).astype(bf16)
        kn2 = jnp.dot(k2, ind_k(), preferred_element_type=f32)
        kn2 = jnp.max(kn2.reshape(RC // 16, 8, 128), axis=0)
        kmax = kn2 if kmax is None else jnp.maximum(kmax, kn2)
        lane = jax.lax.broadcasted_iota(i32, (RC, 128), 1)
        g0 = GBASE[r * CPR]
        for j in range(NSLAB):
            jt = min(j, 4)
            kj = kk[:, jt * 128:(jt + 1) * 128]
            if 1 <= j <= 4:
                kj = jnp.where(lane >= 128 - 8 * j, kk[:, (j - 1) * 128:j * 128], kj)
            kj = jnp.where(lane == ONES_LANE[j], 1.0, kj).astype(bf16)
            k_s[j, pl.ds(r * (RC // 2), RC // 2), :] = pltpu.bitcast(kj, u32)
            rows = []
            for cc in range(CPR):
                for g in range(NGRP[r * CPR + cc]):
                    a = cc * CK + CK - 16 * (g + 1)
                    rows.append(kj[a:a + 16, :])
            ko = jnp.concatenate(rows, axis=0).astype(f32)
            for h in range(6 * j, min(6 * j + 6, H)):
                lo = (DH * h) % 128
                koff_s[h, g0 * 16:(g0 + len(rows)) * 16, :] = pltpu.roll(ko, 128 - lo, axis=1) if lo else ko
        return kmax

    def qproj(r, side):
        xn = xn_chunk(r)
        mg = HG * DH
        row16 = jax.lax.broadcasted_iota(i32, (16, RC), 0)
        row24 = jax.lax.broadcasted_iota(i32, (24, RC), 0)
        for gq in range(H // HG):
            qt = jax.lax.dot_general(wqvt_s[gq * mg:(gq + 1) * mg, :], xn, (((1,), (1,)), ((), ())),
                                     preferred_element_type=f32) * (DH ** -0.5 * LOG2E)
            side(qt)
            qr = qt.astype(bf16).astype(f32)
            for h in range(gq * HG, (gq + 1) * HG):
                base = (DH * h // 8) * 8 - gq * mg
                win = qr[base:base + 24, :]
                brow, v0 = (20, 0) if h % 2 == 0 else (0, 4)
                wm = jnp.where((row24 >= v0) & (row24 < v0 + DH), win, 0.0)
                qn2 = jnp.sum(wm * wm, axis=0, keepdims=True)
                kc = jnp.concatenate([kcol_s[h:h + 1, :]] * (RC // 128), axis=1)
                nbh = (SHIFT - jnp.sqrt(qn2 * kc) * 1.02).astype(bf16).astype(f32)
                qw_s[r * H + h] = jnp.where(row24 == brow, nbh, win)
                t0, tq, ot = q_tiles(h)
                orow = ONES_LANE[h // 6] % 16
                for e in range(2):
                    a = (t0 + e) * 16
                    dim = row16 + a
                    blk = jnp.where((dim >= DH * h) & (dim < DH * h + DH), qr[a - gq * mg:a - gq * mg + 16, :], 0.0)
                    if tq[e] == ot:
                        blk = jnp.where(row16 == orow, nbh, blk)
                    qm_s[r * H + h, 8 * tq[e]:8 * tq[e] + 8, :] = pltpu.bitcast(blk.astype(bf16), u32)
                if ot not in tq:
                    qm_s[r * H + h, 8 * ot:8 * ot + 8, :] = pltpu.bitcast(
                        jnp.where(row16 == orow, nbh, 0.0).astype(bf16), u32)

    def vproj(r, wvt=None, side=None, hg=HG):
        xn = xn_chunk(r)
        mg = hg * DH
        row24 = jax.lax.broadcasted_iota(i32, (24, RC), 0)
        for gq in range(H // hg):
            w = wqvt_s[D + gq * mg:D + (gq + 1) * mg, :] if wvt is None else wvt[gq * mg:(gq + 1) * mg, :]
            vt = jax.lax.dot_general(w, xn, (((1,), (1,)), ((), ())), preferred_element_type=f32)
            if side is not None:
                side(vt)
            vt = vt.astype(bf16).astype(f32)
            vmax_s[...] = jnp.maximum(vmax_s[...], jnp.max(jnp.abs(vt).reshape(mg // 8, 8, RC), axis=0))
            for h in range(gq * hg, (gq + 1) * hg):
                base = (DH * h // 8) * 8 - gq * mg
                ones_row = 20 if h % 2 == 0 else 0
                vt_s[r, h] = jnp.where(row24 == ones_row, 1.0, vt[base:base + 24, :])

    def build_kb(h, par, d, gs, tok):
        for g in gs:
            for half in range(2):
                st = g * 16 + half * 8
                ko = gate(koff_s[h, pl.ds(st if isinstance(st, int) else pl.multiple_of(st, 8), 8), :], tok)
                kbuf[par][g, d, half * 8:half * 8 + 8, :] = jnp.broadcast_to(ko[:, d:d + 1], (8, 128))

    state['neg'] = flag_s[1]
    zero_s[...] = jnp.zeros(zero_s.shape, f32)
    acc_s[...] = jnp.zeros(acc_s.shape, f32)
    vmax_s[...] = jnp.zeros(vmax_s.shape, f32)
    for pb in pbufs:
        pb[...] = jnp.zeros(pb.shape, u32)

    def zfill(r, carry):
        for h in range(H):
            _, tq, ot = q_tiles(h)
            for tt in range(8):
                if tt not in tq and tt != ot:
                    qm_s[r * H + h, 8 * tt:8 * tt + 8, :] = jnp.zeros((8, TQ), u32)
        return carry

    jax.lax.fori_loop(0, NR, zfill, 0)
    cp_x0.wait()
    ln(0)
    cp_wk.wait()
    kmax = kproj(0, None)
    cp_wv.wait()
    cp_x1.wait()
    for c in late(0) + late(1) + [cp_wo]:
        c.start()
    wvt = wv_s[...].T
    wqvt_s[D:2 * D, :] = wvt
    vproj(0, wvt, hg=16)
    ln(1)
    kmax = kproj(1, kmax)
    cp_xr.wait()
    cp_wq.wait()
    vproj(1, hg=16)
    ln(2)
    kmax = kproj(2, kmax)
    wqvt_s[0:D, :] = wq_s[...].T
    ln(3)
    kmax = kproj(3, kmax)
    krow = jnp.max(kmax, axis=0, keepdims=True)
    kcol_s[...] = jnp.broadcast_to(krow, (128, 128)).T[0:H, :]

    def qvloop(i, carry):
        for c in late(i):
            c.wait()
        jobs = []
        kr = pl.ds(pl.multiple_of(i * (D // 2), D // 2), D // 2)
        kr2 = pl.ds(pl.multiple_of(i * (D // 4), D // 4), D // 4)
        fr = pl.ds(pl.multiple_of(i * (F // 2), F // 2), F // 2)
        fr2 = pl.ds(pl.multiple_of(i * (F // 4), F // 4), F // 4)
        for j in range(12):
            def job_g(tok, j=j):
                o = (j % 2) * 128
                wgu_p[j // 2, kr2, o:o + 128] = gate(pltpu.bitcast(wg_s[kr, j * 128:(j + 1) * 128], u32), tok)

            def job_u(tok, j=j):
                o = 256 + (j % 2) * 128
                wgu_p[j // 2, kr2, o:o + 128] = gate(pltpu.bitcast(wu_s[kr, j * 128:(j + 1) * 128], u32), tok)
            jobs += [job_g, job_u]
        for n in range(5):
            def job_d(tok, n=n):
                wd_p[n, fr2, :] = gate(pltpu.bitcast(wd_s[fr, n * 128:(n + 1) * 128], u32), tok)
            jobs.append(job_d)
        for d in range(DH):
            def job_k(tok, d=d):
                build_kb(0, 0, d, [i * (NB // 2) + g for g in range((NB + 1) // 2)], tok)
            jobs.insert(2 * d + 1, job_k)
        nside = 3 * (H // HG) - 1
        cnt = [0]

        def side(res):
            k = cnt[0]
            cnt[0] += 1
            mine = jobs[(k * len(jobs)) // nside:((k + 1) * len(jobs)) // nside] if k < nside else []
            for n, job in enumerate(mine):
                rr = (n * HG * DH // len(mine)) // 8 * 8
                job(res[rr:rr + 8, 0:128])

        qproj(2 * i, side)
        qproj(2 * i + 1, side)
        vproj(2 + i, None, side)
        return carry

    jax.lax.fori_loop(0, 2, qvloop, 0)

    def opaque_zero():
        state['cnt'] += 1
        return (state['h'] + state['cnt']) >> 20

    def vpu_block(h, par, i, tok):
        qt, c, j, t = BLIST[i]
        u = qt * NCK + c
        z0 = opaque_zero()
        qi = qt * H + h + z0
        row = lambda d: d if par == 0 else (d + 4) % 24
        lanes = slice(t * 128, (t + 1) * 128)
        acc = jnp.broadcast_to(qw_s[qi, row(DH):row(DH) + 1, lanes], (16, 128))
        for d in range(DH):
            kb = kbuf[par][GBASE[c] + j + z0, d]
            qb = qw_s[qi, row(d):row(d) + 1, lanes]
            if d == GATE:
                qb = gate(jnp.broadcast_to(qb, (8, 128)), tok)
                qb = jnp.concatenate([qb, qb], axis=0)
            acc = acc + kb * qb
        r0 = (CK - 16 * (j + 1)) // 2
        pbufs[u % NPB][r0:r0 + 8, lanes] = pltpu.bitcast(jnp.exp2(acc).astype(bf16), u32)

    def qk_unit(h, u):
        qt, c = divmod(u, NCK)
        nm = CK - 16 * NGRP[c]
        kc = pltpu.bitcast(k_s[h // 6, pl.ds(c * (CK // 2), nm // 2), :], bf16)
        s = jnp.dot(kc, pltpu.bitcast(qm_s[qt * H + h], bf16), preferred_element_type=f32)
        pbufs[u % NPB][pl.ds(0, nm // 2), :] = pltpu.bitcast(jnp.exp2(s).astype(bf16), u32)
        return [s[r:r + 8, 0:128] for r in range(0, nm, 8)]

    def pv_unit(h, u, acc, zp):
        kc = (u % NCK) * CK
        p = pltpu.bitcast(pbufs[u % NPB][pl.ds(zp, 64), :], bf16)
        o = jnp.dot(vt_s[kc // RC, h, :, pl.ds(kc % RC, CK)], p, preferred_element_type=f32)
        return acc + o, [o[r:r + 8, 0:128] for r in range(0, 24, 8)]

    def ffn_piece(h, p, side):
        kind, j = p
        z0 = opaque_zero()
        acc = None
        for sidx in range(NSUB[kind]):
            if kind == 'gu':
                rows = pl.ds(pl.multiple_of((h + z0) * (FM // 2), FM // 2), FM // 2)
                a = pltpu.bitcast(xn_s[rows, sidx * 128:(sidx + 1) * 128], bf16)
                w = pltpu.bitcast(wgu_p[j, sidx * 64:(sidx + 1) * 64, :], bf16)
            else:
                a = pltpu.bitcast(hh_s[pl.ds(pl.multiple_of(z0 * 8, 8), FM // 2), sidx * 512:(sidx + 1) * 512], bf16)
                w = pltpu.bitcast(wd_p[j, sidx * 256:(sidx + 1) * 256, :], bf16)
            o = jnp.dot(a, w, preferred_element_type=f32)
            acc = o if acc is None else acc + o
            side(sidx * FT, [o[ti * (FM // FT):ti * (FM // FT) + 8, 0:128] for ti in range(FT)])
        if kind == 'gu':
            g = acc[:, :256]
            u = acc[:, 256:]
            hh = (g * u) * (0.5 * jnp.tanh(0.5 * g) + 0.5)
            hh_s[:, j * 256:(j + 1) * 256] = pltpu.bitcast(hh.astype(bf16), u32)
        else:
            y_s[pl.ds(pl.multiple_of(h * FM, FM), FM), j * 128:(j + 1) * 128] = acc

    def block(h, par):
        state['h'] = h
        state['neg'] = h >> 20
        zp = pl.multiple_of((h >> 20) * 8, 8)
        hp = jnp.maximum(h - 1, 0)
        hn = jnp.minimum(h + 1, H - 1)
        acc = acc_s[...]

        def side(k0, toks):
            for ti, tok in enumerate(toks):
                idxs = KASSIGN[k0 + ti]
                for d in sorted(set(i // NB for i in idxs)):
                    build_kb(hn, 1 - par, d, [i % NB for i in idxs if i // NB == d], tok)
                for i in ASSIGN[k0 + ti]:
                    vpu_block(h, par, i, tok)

        for v in range(UPH):
            u = v - LEAD
            side(TOK0[(v, 'qk')], qk_unit(h if u >= 0 else hp, u % UPH))
            w = u - LAGU
            hw = h if w >= 0 else hp
            qt, c = divmod(w % UPH, NCK)
            if c == 0:
                acc = zero_s[h >> 20]
            acc, toks = pv_unit(hw, w % UPH, acc, zp)
            side(TOK0[(v, 'pv')], toks)
            if c == NCK - 1:
                oraw_s[hw * NQ + qt] = acc
            if v in PPOS:
                ffn_piece(h, PPOS[v], lambda o, toks: side(TOK0[(v, 'ffn')] + o, toks))
        acc_s[...] = acc

    def body(b, carry):
        pl.when((b >> 20) == 0)(lambda: block(2 * b, 0))
        pl.when((b >> 21) == 0)(lambda: block(2 * b + 1, 1))
        return carry

    jax.lax.fori_loop(0, H // 2, body, 0)

    cp_wo.wait()
    for u in range(UPH - LEAD, UPH):
        qk_unit(H - 1, u)
    acc = acc_s[...]
    for w in range(UPH - LEAD - LAGU, UPH):
        acc, _ = pv_unit(H - 1, w, acc, 0)
    oraw_s[H * NQ - 1] = acc

    def fallback():
        def item(it, carry):
            h = it // NQ
            qt = it % NQ
            w = pltpu.bitcast(qm_s[qt * H + h], bf16)

            def p1(c, m):
                kc = pltpu.bitcast(k_s[h // 6, pl.ds(pl.multiple_of(c * (CK // 2), CK // 2), CK // 2), :], bf16)
                s = jnp.dot(kc, w, preferred_element_type=f32)
                sfb_s[pl.ds(pl.multiple_of(c * CK, CK), CK), :] = s
                return jnp.maximum(m, jnp.max(s.reshape(CK // 8, 8, TQ), axis=0))
            m = jax.lax.fori_loop(0, NCK, p1, jnp.full((8, TQ), -jnp.inf, f32))
            m = jnp.max(m, axis=0, keepdims=True)

            def p2(r, acc):
                s = sfb_s[pl.ds(pl.multiple_of(r * RC, RC), RC), :]
                p = jnp.exp2(s - m).astype(bf16)
                return acc + jnp.dot(vt_s[r, h], p, preferred_element_type=f32)
            oraw_s[it] = jax.lax.fori_loop(0, NR, p2, jnp.zeros((24, TQ), f32))
            return carry
        jax.lax.fori_loop(0, H * NQ, item, 0)

    def out_copy(t):
        return pltpu.make_async_copy(out_s.at[pl.ds(t * TO, TO), :], o_hbm.at[pl.ds(t * TO, TO), :], sem_out.at[t])

    def tail(qt, carry):
        lo, hi = carry
        row8 = jax.lax.broadcasted_iota(i32, (8, TQ), 0)

        def bcast(ref_row):
            return jnp.concatenate([jnp.broadcast_to(ref_row(slice(n * 128, (n + 1) * 128)), (8, 128))
                                    for n in range(TQ // 128)], axis=1)

        pieces = []
        for g8 in range(H // 8):
            lst = None
            for k in range(8):
                h = g8 * 8 + k
                lrow = 20 if h % 2 == 0 else 0
                lk = bcast(lambda ln_: oraw_s[h * NQ + qt, lrow:lrow + 1, ln_])
                lst = lk if lst is None else jnp.where(row8 == k, lk, lst)
            lo = jnp.minimum(lo, lst)
            hi = jnp.maximum(hi, lst)
            rinv_s[g8 * 8:(g8 + 1) * 8, :] = 1.0 / lst
            for g in range(g8 * 4, g8 * 4 + 4):
                ra = bcast(lambda ln_: rinv_s[2 * g:2 * g + 1, ln_])
                rb = bcast(lambda ln_: rinv_s[2 * g + 1:2 * g + 2, ln_])
                a = oraw_s[2 * g * NQ + qt]
                b = oraw_s[(2 * g + 1) * NQ + qt]
                pieces += [a[0:8] * ra, a[8:16] * ra,
                           jnp.where(row8 < 4, a[16:24] * ra, b[0:8] * rb), b[8:16] * rb, b[16:24] * rb]
        ot = jnp.concatenate(pieces, axis=0).astype(bf16)
        for e in range(TQ // TO):
            rows = pl.ds(pl.multiple_of(qt * TQ + e * TO, TO), TO)
            acc = x_s[rows, :].astype(f32) + y_s[rows, :]
            acc = acc + jax.lax.dot_general(ot[:, e * TO:(e + 1) * TO], wo_s[...], (((0,), (0,)), ((), ())),
                                            preferred_element_type=f32)
            out_s[rows, :] = acc.astype(bf16)
            pltpu.make_async_copy(out_s.at[rows, :], o_hbm.at[rows, :], sem_out.at[qt * (TQ // TO) + e]).start()
        return lo, hi

    def one_pass(p, carry):
        @pl.when(jnp.logical_or(p == 0, flag_s[0] != 0))
        def _():
            lo, hi = jax.lax.fori_loop(0, NQ, tail, (jnp.ones((8, TQ), f32), jnp.ones((8, TQ), f32)))
            vm = jnp.maximum(jnp.max(vmax_s[...]), 1.0)
            ok = (lo >= L_MIN) & (hi * vm <= L_MAX)
            flag_s[0] = (jnp.max(jnp.where(ok, 0.0, 1.0)) > 0.0).astype(i32)
            for t in range(S // TO):
                out_copy(t).wait()
            pl.when(jnp.logical_and(p == 0, flag_s[0] != 0))(fallback)
        return carry

    jax.lax.fori_loop(0, 2, one_pass, 0)


@jax.jit
def pallas_parallel_sum__mha_block__swiglu_ffn__prompt_kernel(A_x, A_wqkv, A_wo, B_x, B_w_gate, B_w_up, B_w_down):
    x = A_x.reshape(S, D)
    bf16 = jnp.bfloat16
    f32 = jnp.float32
    u32 = jnp.uint32
    anyspec = pl.BlockSpec(memory_space=pl.ANY)
    out = pl.pallas_call(
        _kernel,
        in_specs=[anyspec] * 6,
        out_specs=anyspec,
        out_shape=jax.ShapeDtypeStruct((S, D), bf16),
        scratch_shapes=[
            pltpu.VMEM((S, D), bf16),
            pltpu.VMEM((D, D), bf16),
            pltpu.VMEM((D, D), bf16),
            pltpu.VMEM((D, D), bf16),
            pltpu.VMEM((D, D), bf16),
            pltpu.VMEM((D, F), bf16),
            pltpu.VMEM((D, F), bf16),
            pltpu.VMEM((F, D), bf16),
            pltpu.VMEM((S, D), bf16),
            pltpu.VMEM((S // 2, D), u32),
            pltpu.VMEM((2 * D, D), bf16),
            pltpu.VMEM((NSLAB, S // 2, 128), u32),
            pltpu.VMEM((NQ * H, 64, TQ), u32),
            pltpu.VMEM((NR, H, 24, RC), f32),
            pltpu.VMEM((H * NQ, 24, TQ), f32),
            pltpu.VMEM((H, NB * 16, 128), f32),
            pltpu.VMEM((NQ * H, 24, TQ), f32),
            pltpu.VMEM((NB, DH, 16, 128), f32),
            pltpu.VMEM((NB, DH, 16, 128), f32),
            pltpu.VMEM((6, D // 2, 512), u32),
            pltpu.VMEM((5, F // 2, 128), u32),
            pltpu.VMEM((FM // 2, F), u32),
            pltpu.VMEM((S, D), f32),
            pltpu.VMEM((1, 24, TQ), f32),
            pltpu.VMEM((24, TQ), f32),
            pltpu.VMEM((H, 128), f32),
            pltpu.VMEM((8, RC), f32),
            pltpu.VMEM((H, TQ), f32),
            pltpu.SMEM((2,), jnp.int32),
            pltpu.VMEM((S, TQ), f32),
            pltpu.SemaphoreType.DMA((13,)),
            pltpu.SemaphoreType.DMA((S // TO,)),
        ] + [pltpu.VMEM((64, TQ), u32)] * NPB,
        compiler_params=pltpu.CompilerParams(
            vmem_limit_bytes=116 * 1024 * 1024),
        name="fused_block",
    )(x, A_wqkv, A_wo, B_w_gate, B_w_up, B_w_down)
    return out.reshape(1, S, D)
```

```python
import bisect

import jax
import jax.numpy as jnp
import jax.experimental.pallas as pl
import jax.experimental.pallas.tpu as pltpu

S = 2048
D = 640
H = 32
DH = 20
F = 1536
EPS = 1e-5
NSLAB = 6
LOG2E = 1.4426950408889634
SHIFT = 100.0
L_MIN = 2.0 ** -80
L_MAX = 2.0 ** 124

TQ = 512
CK = 128
NCK = S // CK
NQ = S // TQ
RC = 512
NR = S // RC
CPR = RC // CK
TO = 256
NB = 22
GATE = DH - 1
LAGU = 2
LEAD = 1
NPB = 8
FM = S // H
FT = 8
HG = 4

NGRP = [((c + 1) * NB) // NCK - (c * NB) // NCK for c in range(NCK)]
GBASE = [(c * NB) // NCK for c in range(NCK)]
UPH = NQ * NCK
BLIST = [(qt, c, j, t) for qt in range(NQ) for c in range(NCK) for j in range(NGRP[c]) for t in range(4)]


def _plan():
    pieces = [('gu', j) for j in range(6)] + [('dn', n) for n in range(5)]
    nsub = {'gu': 5, 'dn': 3}
    ppos = {2 + (i * (UPH - 4)) // len(pieces): p for i, p in enumerate(pieces)}
    ttime, tunit, tok0 = [], [], {}
    t = 0
    for v in range(UPH):
        nm = CK - 16 * NGRP[(v - LEAD) % NCK]
        tok0[(v, 'qk')] = len(ttime)
        for ti in range(nm // 8):
            ttime.append(t + ti * 8)
            tunit.append(v)
        t += nm
        tok0[(v, 'pv')] = len(ttime)
        for ti in range(3):
            ttime.append(t + ti * 8)
            tunit.append(v + 1)
        t += 24
        if v in ppos:
            tok0[(v, 'ffn')] = len(ttime)
            for _ in range(nsub[ppos[v][0]]):
                for ti in range(FT):
                    ttime.append(t + ti * (FM // FT))
                    tunit.append(v + 1)
                t += FM
    assign = [[] for _ in ttime]
    kassign = [[] for _ in ttime]
    for i, (qt, c, _, _) in enumerate(BLIST):
        k = min(bisect.bisect_left(ttime, (i - 1.0) * t / len(BLIST)), len(ttime) - 1)
        assign[k].append(i)
        u = qt * NCK + c
        assert u - (NPB - LAGU - LEAD - 1) <= tunit[k] <= u + LEAD + LAGU - 1
    nk = DH * NB
    for i in range(nk):
        kassign[bisect.bisect_left(ttime, i * (t - 270) / nk)].append(i)
    hassign = [[] for _ in ttime]
    for i in range(len(HLIST)):
        hassign[bisect.bisect_left(ttime, 300 + (i // 2 * 2) * (t - 600) / len(HLIST))].append(HLIST[i])
    return ppos, nsub, tok0, assign, kassign, hassign


HLIST = [c * (CK // 16) + n for c in range(NCK) for n in range(CK // 16 - NGRP[c])]
PPOS, NSUB, TOK0, ASSIGN, KASSIGN, HASSIGN = _plan()


def _kernel(x_hbm, wqkv_hbm, wo_hbm, wg_hbm, wu_hbm, wd_hbm, o_hbm,
            x_s, wq_s, wk_s, wv_s, wo_s, wg_s, wu_s, wd_s, out_s,
            xn_s, wqvt_s, k_s, qm_s, vt_s, oraw_s, koff_s, qw_s, kb_a, kb_b, kh_a, kh_b,
            wgu_p, wd_p, hh_s, y_s, zero_s, acc_s, kcol_s, vmax_s, rinv_s, flag_s, sfb_s,
            sem_in, sem_out, *pbufs):
    f32 = jnp.float32
    bf16 = jnp.bfloat16
    u32 = jnp.uint32
    i32 = jnp.int32
    kbuf = (kb_a, kb_b)
    khbuf = (kh_a, kh_b)

    cp_x0 = pltpu.make_async_copy(x_hbm.at[pl.ds(0, RC), :], x_s.at[pl.ds(0, RC), :], sem_in.at[0])
    cp_wk = pltpu.make_async_copy(wqkv_hbm.at[:, pl.ds(D, D)], wk_s, sem_in.at[1])
    cp_wq = pltpu.make_async_copy(wqkv_hbm.at[:, pl.ds(0, D)], wq_s, sem_in.at[2])
    cp_wv = pltpu.make_async_copy(wqkv_hbm.at[:, pl.ds(2 * D, D)], wv_s, sem_in.at[3])
    cp_x1 = pltpu.make_async_copy(x_hbm.at[pl.ds(RC, RC), :], x_s.at[pl.ds(RC, RC), :], sem_in.at[4])
    cp_xr = pltpu.make_async_copy(x_hbm.at[pl.ds(2 * RC, 2 * RC), :], x_s.at[pl.ds(2 * RC, 2 * RC), :],
                                  sem_in.at[5])
    cp_wo = pltpu.make_async_copy(wo_hbm, wo_s, sem_in.at[6])

    def late(i):
        cps = []
        for n, (src, dst) in enumerate(((wg_hbm, wg_s), (wu_hbm, wu_s), (wd_hbm, wd_s))):
            hr = src.shape[0] // 2
            rows = pl.ds(i * hr if isinstance(i, int) else pl.multiple_of(i * hr, hr), hr)
            cps.append(pltpu.make_async_copy(src.at[rows, :], dst.at[rows, :], sem_in.at[7 + 3 * i + n]))
        return cps

    for c in (cp_x0, cp_wk, cp_wv, cp_x1, cp_xr, cp_wq):
        c.start()
    flag_s[0] = 0
    flag_s[1] = 0

    state = dict(h=0, cnt=0, neg=0)

    def gate(val, tok):
        r, c = val.shape
        mask = jax.lax.broadcasted_iota(i32, (r, c), 1) < state['neg']
        t = tok if val.dtype == tok.dtype else pltpu.bitcast(tok, val.dtype)
        t = jnp.concatenate([jnp.concatenate([t] * (c // 128), axis=1)] * (r // 8), axis=0)
        return jnp.where(mask, t, val)

    def xn_chunk(r):
        start = r * (RC // 2)
        if not isinstance(r, int):
            start = pl.multiple_of(start, RC // 2)
        return pltpu.bitcast(xn_s[pl.ds(start, RC // 2), :], bf16)

    def ln(r):
        x = x_s[pl.ds(r * RC, RC), :].astype(f32)
        mu = jnp.mean(x, axis=-1, keepdims=True)
        xc = x - mu
        var = jnp.mean(xc * xc, axis=-1, keepdims=True)
        xn_s[pl.ds(r * (RC // 2), RC // 2), :] = pltpu.bitcast((xc * jax.lax.rsqrt(var + EPS)).astype(bf16), u32)

    def ind_k():
        l = jax.lax.broadcasted_iota(i32, (D, 128), 0)
        h = jax.lax.broadcasted_iota(i32, (D, 128), 1)
        return jnp.where((l >= DH * h) & (l < DH * h + DH), 1.0, 0.0).astype(bf16)

    def kproj(r, kmax):
        kk = jnp.dot(xn_chunk(r), wk_s[...], preferred_element_type=f32)
        k2 = kk * kk
        k2 = jnp.maximum(k2[0:RC // 2], k2[RC // 2:RC]).astype(bf16)
        kn2 = jnp.dot(k2, ind_k(), preferred_element_type=f32)
        kn2 = jnp.max(kn2.reshape(RC // 16, 8, 128), axis=0)
        kmax = kn2 if kmax is None else jnp.maximum(kmax, kn2)
        lane = jax.lax.broadcasted_iota(i32, (RC, 128), 1)
        g0 = GBASE[r * CPR]
        for j in range(NSLAB):
            jt = min(j, 4)
            kj = kk[:, jt * 128:(jt + 1) * 128]
            if 1 <= j <= 4:
                kj = jnp.where(lane >= 128 - 8 * j, kk[:, (j - 1) * 128:j * 128], kj)
            kj = kj.astype(bf16)
            k_s[j, pl.ds(r * (RC // 2), RC // 2), :] = pltpu.bitcast(kj, u32)
            rows = []
            for cc in range(CPR):
                for g in range(NGRP[r * CPR + cc]):
                    a = cc * CK + CK - 16 * (g + 1)
                    rows.append(kj[a:a + 16, :])
            ko = jnp.concatenate(rows, axis=0).astype(f32)
            for h in range(6 * j, min(6 * j + 6, H)):
                lo = (DH * h) % 128
                koff_s[h, g0 * 16:(g0 + len(rows)) * 16, :] = pltpu.roll(ko, 128 - lo, axis=1) if lo else ko
        return kmax

    def qproj(r, side):
        xn = xn_chunk(r)
        mg = HG * DH
        row24 = jax.lax.broadcasted_iota(i32, (24, RC), 0)
        zpad = jnp.zeros((8, RC), f32)
        for gq in range(H // HG):
            qt = jax.lax.dot_general(wqvt_s[gq * mg:(gq + 1) * mg, :], xn, (((1,), (1,)), ((), ())),
                                     preferred_element_type=f32) * (DH ** -0.5 * LOG2E)
            side(qt)
            qr = qt.astype(bf16).astype(f32)
            for h in range(gq * HG, (gq + 1) * HG):
                base = (DH * h // 8) * 8 - gq * mg
                win = qr[base:base + 24, :]
                brow, v0 = (20, 0) if h % 2 == 0 else (0, 4)
                wm = jnp.where((row24 >= v0) & (row24 < v0 + DH), win, 0.0)
                qn2 = jnp.sum(wm * wm, axis=0, keepdims=True)
                kc = jnp.concatenate([kcol_s[h:h + 1, :]] * (RC // 128), axis=1)
                nbh = (SHIFT - jnp.sqrt(qn2 * kc) * 1.02).astype(bf16).astype(f32)
                wb = jnp.where(row24 == brow, nbh, wm)
                qw_s[r * H + h] = wb
                qm_s[r * H + h] = pltpu.bitcast(jnp.concatenate([wb, zpad], axis=0).astype(bf16), u32)

    def vproj(r, wvt=None, side=None, hg=HG):
        xn = xn_chunk(r)
        mg = hg * DH
        row24 = jax.lax.broadcasted_iota(i32, (24, RC), 0)
        for gq in range(H // hg):
            w = wqvt_s[D + gq * mg:D + (gq + 1) * mg, :] if wvt is None else wvt[gq * mg:(gq + 1) * mg, :]
            vt = jax.lax.dot_general(w, xn, (((1,), (1,)), ((), ())), preferred_element_type=f32)
            if side is not None:
                side(vt)
            vt = vt.astype(bf16).astype(f32)
            vmax_s[...] = jnp.maximum(vmax_s[...], jnp.max(jnp.abs(vt).reshape(mg // 8, 8, RC), axis=0))
            for h in range(gq * hg, (gq + 1) * hg):
                base = (DH * h // 8) * 8 - gq * mg
                ones_row = 20 if h % 2 == 0 else 0
                vt_s[r, h] = jnp.where(row24 == ones_row, 1.0, vt[base:base + 24, :])

    def build_kb(h, par, d, gs, tok):
        for g in gs:
            for half in range(2):
                st = g * 16 + half * 8
                ko = gate(koff_s[h, pl.ds(st if isinstance(st, int) else pl.multiple_of(st, 8), 8), :], tok)
                kbuf[par][g, d, half * 8:half * 8 + 8, :] = jnp.broadcast_to(ko[:, d:d + 1], (8, 128))

    def build_kh(h, par, tiles, tok):
        brow, v0 = (20, 0) if par == 0 else (0, 4)
        lane = jax.lax.broadcasted_iota(i32, (8, 128), 1)
        ones = gate(jnp.full((8, 128), 0x3F803F80, u32), tok)
        sh = (v0 - DH * h) % 128
        for t in tiles:
            rows = pl.ds(t * 8 if isinstance(t, int) else pl.multiple_of(t * 8, 8), 8)
            kt = k_s[h // 6, rows, :]
            if not (isinstance(sh, int) and sh == 0):
                kt = pltpu.roll(kt, sh, axis=1)
            khbuf[par][rows, :] = jnp.where(lane == brow, ones, kt)

    state['neg'] = flag_s[1]
    kh_b[...] = jnp.zeros(kh_b.shape, u32)
    zero_s[...] = jnp.zeros(zero_s.shape, f32)
    acc_s[...] = jnp.zeros(acc_s.shape, f32)
    vmax_s[...] = jnp.zeros(vmax_s.shape, f32)
    for pb in pbufs:
        pb[...] = jnp.zeros(pb.shape, u32)

    cp_x0.wait()
    ln(0)
    cp_wk.wait()
    kmax = kproj(0, None)
    cp_wv.wait()
    cp_x1.wait()
    for c in late(0) + late(1) + [cp_wo]:
        c.start()
    wvt = wv_s[...].T
    wqvt_s[D:2 * D, :] = wvt
    vproj(0, wvt, hg=16)
    ln(1)
    kmax = kproj(1, kmax)
    cp_xr.wait()
    cp_wq.wait()
    vproj(1, hg=16)
    ln(2)
    kmax = kproj(2, kmax)
    wqvt_s[0:D, :] = wq_s[...].T
    ln(3)
    kmax = kproj(3, kmax)
    krow = jnp.max(kmax, axis=0, keepdims=True)
    kcol_s[...] = jnp.broadcast_to(krow, (128, 128)).T[0:H, :]

    def qvloop(i, carry):
        for c in late(i):
            c.wait()
        jobs = []
        kr = pl.ds(pl.multiple_of(i * (D // 2), D // 2), D // 2)
        kr2 = pl.ds(pl.multiple_of(i * (D // 4), D // 4), D // 4)
        fr = pl.ds(pl.multiple_of(i * (F // 2), F // 2), F // 2)
        fr2 = pl.ds(pl.multiple_of(i * (F // 4), F // 4), F // 4)
        for j in range(12):
            def job_g(tok, j=j):
                o = (j % 2) * 128
                wgu_p[j // 2, kr2, o:o + 128] = gate(pltpu.bitcast(wg_s[kr, j * 128:(j + 1) * 128], u32), tok)

            def job_u(tok, j=j):
                o = 256 + (j % 2) * 128
                wgu_p[j // 2, kr2, o:o + 128] = gate(pltpu.bitcast(wu_s[kr, j * 128:(j + 1) * 128], u32), tok)
            jobs += [job_g, job_u]
        for n in range(5):
            def job_d(tok, n=n):
                wd_p[n, fr2, :] = gate(pltpu.bitcast(wd_s[fr, n * 128:(n + 1) * 128], u32), tok)
            jobs.append(job_d)
        for d in range(DH):
            def job_k(tok, d=d):
                build_kb(0, 0, d, [i * (NB // 2) + g for g in range((NB + 1) // 2)], tok)
            jobs.insert(2 * d + 1, job_k)
        for n in range(4):
            def job_h(tok, n=n):
                build_kh(0, 0, [i * 64 + n * 16 + t for t in range(16)], tok)
            jobs.append(job_h)
        nside = 3 * (H // HG) - 1
        cnt = [0]

        def side(res):
            k = cnt[0]
            cnt[0] += 1
            mine = jobs[(k * len(jobs)) // nside:((k + 1) * len(jobs)) // nside] if k < nside else []
            for n, job in enumerate(mine):
                rr = (n * HG * DH // len(mine)) // 8 * 8
                job(res[rr:rr + 8, 0:128])

        qproj(2 * i, side)
        qproj(2 * i + 1, side)
        vproj(2 + i, None, side)
        return carry

    jax.lax.fori_loop(0, 2, qvloop, 0)

    def opaque_zero():
        state['cnt'] += 1
        return (state['h'] + state['cnt']) >> 20

    def vpu_block(h, par, i, tok):
        qt, c, j, t = BLIST[i]
        u = qt * NCK + c
        z0 = opaque_zero()
        qi = qt * H + h + z0
        row = lambda d: d if par == 0 else (d + 4) % 24
        lanes = slice(t * 128, (t + 1) * 128)
        acc = jnp.broadcast_to(qw_s[qi, row(DH):row(DH) + 1, lanes], (16, 128))
        for d in range(DH):
            kb = kbuf[par][GBASE[c] + j + z0, d]
            qb = qw_s[qi, row(d):row(d) + 1, lanes]
            if d == GATE:
                qb = gate(jnp.broadcast_to(qb, (8, 128)), tok)
                qb = jnp.concatenate([qb, qb], axis=0)
            acc = acc + kb * qb
        r0 = (CK - 16 * (j + 1)) // 2
        pbufs[u % NPB][r0:r0 + 8, lanes] = pltpu.bitcast(jnp.exp2(acc).astype(bf16), u32)

    def qk_unit(h, par, u):
        qt, c = divmod(u, NCK)
        nm = CK - 16 * NGRP[c]
        z0 = opaque_zero() * 8
        if not isinstance(z0, int):
            z0 = pl.multiple_of(z0, 8)
        kc = pltpu.bitcast(khbuf[par][pl.ds(c * (CK // 2) + z0, nm // 2), :], bf16)[:, 0:32]
        s = jnp.dot(kc, pltpu.bitcast(qm_s[qt * H + h], bf16), preferred_element_type=f32)
        pbufs[u % NPB][pl.ds(0, nm // 2), :] = pltpu.bitcast(jnp.exp2(s).astype(bf16), u32)
        return [s[r:r + 8, 0:128] for r in range(0, nm, 8)]

    def pv_unit(h, u, acc, zp):
        kc = (u % NCK) * CK
        p = pltpu.bitcast(pbufs[u % NPB][pl.ds(zp, 64), :], bf16)
        o = jnp.dot(vt_s[kc // RC, h, :, pl.ds(kc % RC, CK)], p, preferred_element_type=f32)
        return acc + o, [o[r:r + 8, 0:128] for r in range(0, 24, 8)]

    def ffn_piece(h, p, side):
        kind, j = p
        z0 = opaque_zero()
        acc = None
        for sidx in range(NSUB[kind]):
            if kind == 'gu':
                rows = pl.ds(pl.multiple_of((h + z0) * (FM // 2), FM // 2), FM // 2)
                a = pltpu.bitcast(xn_s[rows, sidx * 128:(sidx + 1) * 128], bf16)
                w = pltpu.bitcast(wgu_p[j, sidx * 64:(sidx + 1) * 64, :], bf16)
            else:
                a = pltpu.bitcast(hh_s[pl.ds(pl.multiple_of(z0 * 8, 8), FM // 2), sidx * 512:(sidx + 1) * 512], bf16)
                w = pltpu.bitcast(wd_p[j, sidx * 256:(sidx + 1) * 256, :], bf16)
            o = jnp.dot(a, w, preferred_element_type=f32)
            acc = o if acc is None else acc + o
            side(sidx * FT, [o[ti * (FM // FT):ti * (FM // FT) + 8, 0:128] for ti in range(FT)])
        if kind == 'gu':
            g = acc[:, :256]
            u = acc[:, 256:]
            hh = (g * u) * (0.5 * jnp.tanh(0.5 * g) + 0.5)
            hh_s[:, j * 256:(j + 1) * 256] = pltpu.bitcast(hh.astype(bf16), u32)
        else:
            y_s[pl.ds(pl.multiple_of(h * FM, FM), FM), j * 128:(j + 1) * 128] = acc

    def block(h, par):
        state['h'] = h
        state['neg'] = h >> 20
        zp = pl.multiple_of((h >> 20) * 8, 8)
        hp = jnp.maximum(h - 1, 0)
        hn = jnp.minimum(h + 1, H - 1)
        hn2 = jnp.minimum(h + 1, H - 1 - par)
        acc = acc_s[...]

        def side(k0, toks):
            for ti, tok in enumerate(toks):
                idxs = KASSIGN[k0 + ti]
                for d in sorted(set(i // NB for i in idxs)):
                    build_kb(hn, 1 - par, d, [i % NB for i in idxs if i // NB == d], tok)
                if HASSIGN[k0 + ti]:
                    build_kh(hn2, 1 - par, HASSIGN[k0 + ti], tok)
                for i in ASSIGN[k0 + ti]:
                    vpu_block(h, par, i, tok)

        for v in range(UPH):
            u = v - LEAD
            side(TOK0[(v, 'qk')], qk_unit(h, par, u) if u >= 0 else qk_unit(hp, 1 - par, u % UPH))
            w = u - LAGU
            hw = h if w >= 0 else hp
            qt, c = divmod(w % UPH, NCK)
            if c == 0:
                acc = zero_s[h >> 20]
            acc, toks = pv_unit(hw, w % UPH, acc, zp)
            side(TOK0[(v, 'pv')], toks)
            if c == NCK - 1:
                oraw_s[hw * NQ + qt] = acc
            if v in PPOS:
                ffn_piece(h, PPOS[v], lambda o, toks: side(TOK0[(v, 'ffn')] + o, toks))
        acc_s[...] = acc

    def body(b, carry):
        pl.when((b >> 20) == 0)(lambda: block(2 * b, 0))
        pl.when((b >> 21) == 0)(lambda: block(2 * b + 1, 1))
        return carry

    jax.lax.fori_loop(0, H // 2, body, 0)

    cp_wo.wait()
    state['h'] = 0
    for u in range(UPH - LEAD, UPH):
        qk_unit(H - 1, 1, u)
    acc = acc_s[...]
    for w in range(UPH - LEAD - LAGU, UPH):
        acc, _ = pv_unit(H - 1, w, acc, 0)
    oraw_s[H * NQ - 1] = acc

    def fallback():
        def item(it, carry):
            h = it // NQ
            qt = it % NQ
            odd = h % 2
            row24 = jax.lax.broadcasted_iota(i32, (24, TQ), 0)
            w = jnp.where(row24 == 20 - 20 * odd, 0.0, qw_s[qt * H + h])
            w = jnp.concatenate([w, jnp.zeros((8, TQ), f32)], axis=0).astype(bf16)
            sh = (4 * odd - DH * h) % 128

            def p1(c, m):
                kc = pltpu.roll(k_s[h // 6, pl.ds(pl.multiple_of(c * (CK // 2), CK // 2), CK // 2), :], sh, axis=1)
                s = jnp.dot(pltpu.bitcast(kc, bf16)[:, 0:32], w, preferred_element_type=f32)
                sfb_s[pl.ds(pl.multiple_of(c * CK, CK), CK), :] = s
                return jnp.maximum(m, jnp.max(s.reshape(CK // 8, 8, TQ), axis=0))
            m = jax.lax.fori_loop(0, NCK, p1, jnp.full((8, TQ), -jnp.inf, f32))
            m = jnp.max(m, axis=0, keepdims=True)

            def p2(r, acc):
                s = sfb_s[pl.ds(pl.multiple_of(r * RC, RC), RC), :]
                p = jnp.exp2(s - m).astype(bf16)
                return acc + jnp.dot(vt_s[r, h], p, preferred_element_type=f32)
            oraw_s[it] = jax.lax.fori_loop(0, NR, p2, jnp.zeros((24, TQ), f32))
            return carry
        jax.lax.fori_loop(0, H * NQ, item, 0)

    def out_copy(t):
        return pltpu.make_async_copy(out_s.at[pl.ds(t * TO, TO), :], o_hbm.at[pl.ds(t * TO, TO), :], sem_out.at[t])

    def tail(qt, carry):
        lo, hi = carry
        row8 = jax.lax.broadcasted_iota(i32, (8, TQ), 0)

        def bcast(ref_row):
            return jnp.concatenate([jnp.broadcast_to(ref_row(slice(n * 128, (n + 1) * 128)), (8, 128))
                                    for n in range(TQ // 128)], axis=1)

        pieces = []
        for g8 in range(H // 8):
            lst = None
            for k in range(8):
                h = g8 * 8 + k
                lrow = 20 if h % 2 == 0 else 0
                lk = bcast(lambda ln_: oraw_s[h * NQ + qt, lrow:lrow + 1, ln_])
                lst = lk if lst is None else jnp.where(row8 == k, lk, lst)
            lo = jnp.minimum(lo, lst)
            hi = jnp.maximum(hi, lst)
            rinv_s[g8 * 8:(g8 + 1) * 8, :] = 1.0 / lst
            for g in range(g8 * 4, g8 * 4 + 4):
                ra = bcast(lambda ln_: rinv_s[2 * g:2 * g + 1, ln_])
                rb = bcast(lambda ln_: rinv_s[2 * g + 1:2 * g + 2, ln_])
                a = oraw_s[2 * g * NQ + qt]
                b = oraw_s[(2 * g + 1) * NQ + qt]
                pieces += [a[0:8] * ra, a[8:16] * ra,
                           jnp.where(row8 < 4, a[16:24] * ra, b[0:8] * rb), b[8:16] * rb, b[16:24] * rb]
        ot = jnp.concatenate(pieces, axis=0).astype(bf16)
        for e in range(TQ // TO):
            rows = pl.ds(pl.multiple_of(qt * TQ + e * TO, TO), TO)
            acc = x_s[rows, :].astype(f32) + y_s[rows, :]
            acc = acc + jax.lax.dot_general(ot[:, e * TO:(e + 1) * TO], wo_s[...], (((0,), (0,)), ((), ())),
                                            preferred_element_type=f32)
            out_s[rows, :] = acc.astype(bf16)
            pltpu.make_async_copy(out_s.at[rows, :], o_hbm.at[rows, :], sem_out.at[qt * (TQ // TO) + e]).start()
        return lo, hi

    def one_pass(p, carry):
        @pl.when(jnp.logical_or(p == 0, flag_s[0] != 0))
        def _():
            lo, hi = jax.lax.fori_loop(0, NQ, tail, (jnp.ones((8, TQ), f32), jnp.ones((8, TQ), f32)))
            vm = jnp.maximum(jnp.max(vmax_s[...]), 1.0)
            ok = (lo >= L_MIN) & (hi * vm <= L_MAX)
            flag_s[0] = (jnp.max(jnp.where(ok, 0.0, 1.0)) > 0.0).astype(i32)
            for t in range(S // TO):
                out_copy(t).wait()
            pl.when(jnp.logical_and(p == 0, flag_s[0] != 0))(fallback)
        return carry

    jax.lax.fori_loop(0, 2, one_pass, 0)


@jax.jit
def pallas_parallel_sum__mha_block__swiglu_ffn__prompt_kernel(A_x, A_wqkv, A_wo, B_x, B_w_gate, B_w_up, B_w_down):
    x = A_x.reshape(S, D)
    bf16 = jnp.bfloat16
    f32 = jnp.float32
    u32 = jnp.uint32
    anyspec = pl.BlockSpec(memory_space=pl.ANY)
    out = pl.pallas_call(
        _kernel,
        in_specs=[anyspec] * 6,
        out_specs=anyspec,
        out_shape=jax.ShapeDtypeStruct((S, D), bf16),
        scratch_shapes=[
            pltpu.VMEM((S, D), bf16),
            pltpu.VMEM((D, D), bf16),
            pltpu.VMEM((D, D), bf16),
            pltpu.VMEM((D, D), bf16),
            pltpu.VMEM((D, D), bf16),
            pltpu.VMEM((D, F), bf16),
            pltpu.VMEM((D, F), bf16),
            pltpu.VMEM((F, D), bf16),
            pltpu.VMEM((S, D), bf16),
            pltpu.VMEM((S // 2, D), u32),
            pltpu.VMEM((2 * D, D), bf16),
            pltpu.VMEM((NSLAB, S // 2, 128), u32),
            pltpu.VMEM((NQ * H, 16, TQ), u32),
            pltpu.VMEM((NR, H, 24, RC), f32),
            pltpu.VMEM((H * NQ, 24, TQ), f32),
            pltpu.VMEM((H, NB * 16, 128), f32),
            pltpu.VMEM((NQ * H, 24, TQ), f32),
            pltpu.VMEM((NB, DH, 16, 128), f32),
            pltpu.VMEM((NB, DH, 16, 128), f32),
            pltpu.VMEM((S // 2, 128), u32),
            pltpu.VMEM((S // 2, 128), u32),
            pltpu.VMEM((6, D // 2, 512), u32),
            pltpu.VMEM((5, F // 2, 128), u32),
            pltpu.VMEM((FM // 2, F), u32),
            pltpu.VMEM((S, D), f32),
            pltpu.VMEM((1, 24, TQ), f32),
            pltpu.VMEM((24, TQ), f32),
            pltpu.VMEM((H, 128), f32),
            pltpu.VMEM((8, RC), f32),
            pltpu.VMEM((H, TQ), f32),
            pltpu.SMEM((2,), jnp.int32),
            pltpu.VMEM((S, TQ), f32),
            pltpu.SemaphoreType.DMA((13,)),
            pltpu.SemaphoreType.DMA((S // TO,)),
        ] + [pltpu.VMEM((64, TQ), u32)] * NPB,
        compiler_params=pltpu.CompilerParams(
            vmem_limit_bytes=116 * 1024 * 1024),
        name="fused_block",
    )(x, A_wqkv, A_wo, B_w_gate, B_w_up, B_w_down)
    return out.reshape(1, S, D)
```

```python
import bisect

import jax
import jax.numpy as jnp
import jax.experimental.pallas as pl
import jax.experimental.pallas.tpu as pltpu

S = 2048
D = 640
H = 32
DH = 20
F = 1536
EPS = 1e-5
NSLAB = 6
LOG2E = 1.4426950408889634
SHIFT = 100.0
L_MIN = 2.0 ** -80
L_MAX = 2.0 ** 124

TQ = 512
CK = 128
NCK = S // CK
NQ = S // TQ
RC = 512
NR = S // RC
CPR = RC // CK
TO = 256
NB = 23
GATE = DH - 1
LAGU = 3
LEAD = 0
NPB = 8
FM = S // H
FT = 8
HG = 4

NBA = (NB + 1) // 2 * 2
NGRP = [((c + 1) * NB) // NCK - (c * NB) // NCK for c in range(NCK)]
GBASE = [(c * NB) // NCK for c in range(NCK)]
UPH = NQ * NCK
BLIST = [(qt, c, j, t) for qt in range(NQ) for c in range(NCK) for j in range(NGRP[c]) for t in range(4)]


def _plan():
    pieces = [('gu', j) for j in range(6)] + [('dn', n) for n in range(5)]
    nsub = {'gu': 5, 'dn': 3}
    ppos = {4 + (i * (UPH - 8)) // len(pieces): p for i, p in enumerate(pieces)}
    ttime, tunit, tok0 = [], [], {}
    t = 0
    for v in range(UPH):
        nm = CK - 16 * NGRP[(v - LEAD) % NCK]
        tok0[(v, 'qk')] = len(ttime)
        for ti in range(nm // 8):
            ttime.append(t + ti * 8)
            tunit.append(v)
        t += nm
        tok0[(v, 'pv')] = len(ttime)
        for ti in range(3):
            ttime.append(t + ti * 8)
            tunit.append(v + 1)
        t += 24
        if v in ppos:
            tok0[(v, 'ffn')] = len(ttime)
            for _ in range(nsub[ppos[v][0]]):
                for ti in range(FT):
                    ttime.append(t + ti * (FM // FT))
                    tunit.append(v + 1)
                t += FM
    assign = [[] for _ in ttime]
    kassign = [[] for _ in ttime]
    for i, (qt, c, _, _) in enumerate(BLIST):
        k = min(bisect.bisect_left(ttime, (i - 0.5) * t / len(BLIST)), len(ttime) - 1)
        assign[k].append(i)
        u = qt * NCK + c
        assert u - (NPB - LAGU - LEAD - 1) <= tunit[k] <= u + LEAD + LAGU - 1
    nk = DH * NB
    for i in range(nk):
        kassign[bisect.bisect_left(ttime, i * (t - 270) / nk)].append(i)
    hassign = [[] for _ in ttime]
    for i in range(len(HLIST)):
        hassign[bisect.bisect_left(ttime, 300 + (i // 2 * 2) * (t - 600) / len(HLIST))].append(HLIST[i])
    return ppos, nsub, tok0, assign, kassign, hassign


HLIST = [c * (CK // 16) + n for c in range(NCK) for n in range(CK // 16 - NGRP[c])]
PPOS, NSUB, TOK0, ASSIGN, KASSIGN, HASSIGN = _plan()


def _kernel(x_hbm, wqkv_hbm, wo_hbm, wg_hbm, wu_hbm, wd_hbm, o_hbm,
            x_s, wq_s, wk_s, wv_s, wo_s, wg_s, wu_s, wd_s, out_s,
            xn_s, wqvt_s, k_s, qm_s, vt_s, oraw_s, koff_s, qw_s, kb_a, kb_b, kh_a, kh_b,
            wgu_p, wd_p, hh_s, y_s, zero_s, acc_s, kcol_s, vmax_s, rinv_s, flag_s, sfb_s,
            sem_in, sem_out, *pbufs):
    f32 = jnp.float32
    bf16 = jnp.bfloat16
    u32 = jnp.uint32
    i32 = jnp.int32
    kbuf = (kb_a, kb_b)
    khbuf = (kh_a, kh_b)

    cp_x0 = pltpu.make_async_copy(x_hbm.at[pl.ds(0, RC), :], x_s.at[pl.ds(0, RC), :], sem_in.at[0])
    cp_wk = pltpu.make_async_copy(wqkv_hbm.at[:, pl.ds(D, D)], wk_s, sem_in.at[1])
    cp_wq = pltpu.make_async_copy(wqkv_hbm.at[:, pl.ds(0, D)], wq_s, sem_in.at[2])
    cp_wv = pltpu.make_async_copy(wqkv_hbm.at[:, pl.ds(2 * D, D)], wv_s, sem_in.at[3])
    cp_x1 = pltpu.make_async_copy(x_hbm.at[pl.ds(RC, RC), :], x_s.at[pl.ds(RC, RC), :], sem_in.at[4])
    cp_xr = pltpu.make_async_copy(x_hbm.at[pl.ds(2 * RC, 2 * RC), :], x_s.at[pl.ds(2 * RC, 2 * RC), :],
                                  sem_in.at[5])
    cp_wo = pltpu.make_async_copy(wo_hbm, wo_s, sem_in.at[6])

    def late(i):
        cps = []
        for n, (src, dst) in enumerate(((wg_hbm, wg_s), (wu_hbm, wu_s), (wd_hbm, wd_s))):
            hr = src.shape[0] // 2
            rows = pl.ds(i * hr if isinstance(i, int) else pl.multiple_of(i * hr, hr), hr)
            cps.append(pltpu.make_async_copy(src.at[rows, :], dst.at[rows, :], sem_in.at[7 + 3 * i + n]))
        return cps

    for c in (cp_x0, cp_wk, cp_wv, cp_x1, cp_xr, cp_wq):
        c.start()
    flag_s[0] = 0
    flag_s[1] = 0

    state = dict(h=0, cnt=0, neg=0)

    def gate(val, tok):
        r, c = val.shape
        mask = jax.lax.broadcasted_iota(i32, (r, c), 1) < state['neg']
        t = tok if val.dtype == tok.dtype else pltpu.bitcast(tok, val.dtype)
        t = jnp.concatenate([jnp.concatenate([t] * (c // 128), axis=1)] * (r // 8), axis=0)
        return jnp.where(mask, t, val)

    def xn_chunk(r):
        start = r * (RC // 2)
        if not isinstance(r, int):
            start = pl.multiple_of(start, RC // 2)
        return pltpu.bitcast(xn_s[pl.ds(start, RC // 2), :], bf16)

    def ln(r):
        x = x_s[pl.ds(r * RC, RC), :].astype(f32)
        mu = jnp.mean(x, axis=-1, keepdims=True)
        xc = x - mu
        var = jnp.mean(xc * xc, axis=-1, keepdims=True)
        xn_s[pl.ds(r * (RC // 2), RC // 2), :] = pltpu.bitcast((xc * jax.lax.rsqrt(var + EPS)).astype(bf16), u32)

    def ind_k():
        l = jax.lax.broadcasted_iota(i32, (D, 128), 0)
        h = jax.lax.broadcasted_iota(i32, (D, 128), 1)
        return jnp.where((l >= DH * h) & (l < DH * h + DH), 1.0, 0.0).astype(bf16)

    def kproj(r, kmax):
        kk = jnp.dot(xn_chunk(r), wk_s[...], preferred_element_type=f32)
        k2 = kk * kk
        k2 = jnp.maximum(k2[0:RC // 2], k2[RC // 2:RC]).astype(bf16)
        kn2 = jnp.dot(k2, ind_k(), preferred_element_type=f32)
        kn2 = jnp.max(kn2.reshape(RC // 16, 8, 128), axis=0)
        kmax = kn2 if kmax is None else jnp.maximum(kmax, kn2)
        lane = jax.lax.broadcasted_iota(i32, (RC, 128), 1)
        g0 = GBASE[r * CPR]
        for j in range(NSLAB):
            jt = min(j, 4)
            kj = kk[:, jt * 128:(jt + 1) * 128]
            if 1 <= j <= 4:
                kj = jnp.where(lane >= 128 - 8 * j, kk[:, (j - 1) * 128:j * 128], kj)
            kj = kj.astype(bf16)
            k_s[j, pl.ds(r * (RC // 2), RC // 2), :] = pltpu.bitcast(kj, u32)
            rows = []
            for cc in range(CPR):
                for g in range(NGRP[r * CPR + cc]):
                    a = cc * CK + CK - 16 * (g + 1)
                    rows.append(kj[a:a + 16, :])
            ko = jnp.concatenate(rows, axis=0).astype(f32)
            for h in range(6 * j, min(6 * j + 6, H)):
                lo = (DH * h) % 128
                koff_s[h, g0 * 16:(g0 + len(rows)) * 16, :] = pltpu.roll(ko, 128 - lo, axis=1) if lo else ko
        return kmax

    def qproj(r, side):
        xn = xn_chunk(r)
        mg = HG * DH
        row24 = jax.lax.broadcasted_iota(i32, (24, RC), 0)
        zpad = jnp.zeros((8, RC), f32)
        for gq in range(H // HG):
            qt = jax.lax.dot_general(wqvt_s[gq * mg:(gq + 1) * mg, :], xn, (((1,), (1,)), ((), ())),
                                     preferred_element_type=f32) * (DH ** -0.5 * LOG2E)
            side(qt)
            qr = qt.astype(bf16).astype(f32)
            for h in range(gq * HG, (gq + 1) * HG):
                base = (DH * h // 8) * 8 - gq * mg
                win = qr[base:base + 24, :]
                brow, v0 = (20, 0) if h % 2 == 0 else (0, 4)
                wm = jnp.where((row24 >= v0) & (row24 < v0 + DH), win, 0.0)
                qn2 = jnp.sum(wm * wm, axis=0, keepdims=True)
                kc = jnp.concatenate([kcol_s[h:h + 1, :]] * (RC // 128), axis=1)
                nbh = (SHIFT - jnp.sqrt(qn2 * kc) * 1.02).astype(bf16).astype(f32)
                wb = jnp.where(row24 == brow, nbh, wm)
                qw_s[r * H + h] = wb
                qm_s[r * H + h] = pltpu.bitcast(jnp.concatenate([wb, zpad], axis=0).astype(bf16), u32)

    def vproj(r, wvt=None, side=None, hg=HG):
        xn = xn_chunk(r)
        mg = hg * DH
        row24 = jax.lax.broadcasted_iota(i32, (24, RC), 0)
        for gq in range(H // hg):
            w = wqvt_s[D + gq * mg:D + (gq + 1) * mg, :] if wvt is None else wvt[gq * mg:(gq + 1) * mg, :]
            vt = jax.lax.dot_general(w, xn, (((1,), (1,)), ((), ())), preferred_element_type=f32)
            if side is not None:
                side(vt)
            vt = vt.astype(bf16).astype(f32)
            vmax_s[...] = jnp.maximum(vmax_s[...], jnp.max(jnp.abs(vt).reshape(mg // 8, 8, RC), axis=0))
            for h in range(gq * hg, (gq + 1) * hg):
                base = (DH * h // 8) * 8 - gq * mg
                ones_row = 20 if h % 2 == 0 else 0
                vt_s[r, h] = jnp.where(row24 == ones_row, 1.0, vt[base:base + 24, :])

    def build_kb(h, par, d, gs, tok):
        for g in gs:
            for half in range(2):
                st = g * 16 + half * 8
                ko = gate(koff_s[h, pl.ds(st if isinstance(st, int) else pl.multiple_of(st, 8), 8), :], tok)
                kbuf[par][g, d, half * 8:half * 8 + 8, :] = jnp.broadcast_to(ko[:, d:d + 1], (8, 128))

    def build_kh(h, par, tiles, tok):
        brow, v0 = (20, 0) if par == 0 else (0, 4)
        lane = jax.lax.broadcasted_iota(i32, (8, 128), 1)
        ones = gate(jnp.full((8, 128), 0x3F803F80, u32), tok)
        sh = (v0 - DH * h) % 128
        for t in tiles:
            rows = pl.ds(t * 8 if isinstance(t, int) else pl.multiple_of(t * 8, 8), 8)
            kt = k_s[h // 6, rows, :]
            if not (isinstance(sh, int) and sh == 0):
                kt = pltpu.roll(kt, sh, axis=1)
            khbuf[par][rows, :] = jnp.where(lane == brow, ones, kt)

    state['neg'] = flag_s[1]
    kh_b[...] = jnp.zeros(kh_b.shape, u32)
    zero_s[...] = jnp.zeros(zero_s.shape, f32)
    acc_s[...] = jnp.zeros(acc_s.shape, f32)
    vmax_s[...] = jnp.zeros(vmax_s.shape, f32)
    for pb in pbufs:
        pb[...] = jnp.zeros(pb.shape, u32)

    cp_x0.wait()
    ln(0)
    cp_wk.wait()
    kmax = kproj(0, None)
    cp_wv.wait()
    cp_x1.wait()
    for c in late(0) + late(1) + [cp_wo]:
        c.start()
    wvt = wv_s[...].T
    wqvt_s[D:2 * D, :] = wvt
    vproj(0, wvt, hg=16)
    ln(1)
    kmax = kproj(1, kmax)
    cp_xr.wait()
    cp_wq.wait()
    vproj(1, hg=16)
    ln(2)
    kmax = kproj(2, kmax)
    wqvt_s[0:D, :] = wq_s[...].T
    ln(3)
    kmax = kproj(3, kmax)
    krow = jnp.max(kmax, axis=0, keepdims=True)
    kcol_s[...] = jnp.broadcast_to(krow, (128, 128)).T[0:H, :]

    def qvloop(i, carry):
        for c in late(i):
            c.wait()
        jobs = []
        kr = pl.ds(pl.multiple_of(i * (D // 2), D // 2), D // 2)
        kr2 = pl.ds(pl.multiple_of(i * (D // 4), D // 4), D // 4)
        fr = pl.ds(pl.multiple_of(i * (F // 2), F // 2), F // 2)
        fr2 = pl.ds(pl.multiple_of(i * (F // 4), F // 4), F // 4)
        for j in range(12):
            def job_g(tok, j=j):
                o = (j % 2) * 128
                wgu_p[j // 2, kr2, o:o + 128] = gate(pltpu.bitcast(wg_s[kr, j * 128:(j + 1) * 128], u32), tok)

            def job_u(tok, j=j):
                o = 256 + (j % 2) * 128
                wgu_p[j // 2, kr2, o:o + 128] = gate(pltpu.bitcast(wu_s[kr, j * 128:(j + 1) * 128], u32), tok)
            jobs += [job_g, job_u]
        for n in range(5):
            def job_d(tok, n=n):
                wd_p[n, fr2, :] = gate(pltpu.bitcast(wd_s[fr, n * 128:(n + 1) * 128], u32), tok)
            jobs.append(job_d)
        for d in range(DH):
            def job_k(tok, d=d):
                build_kb(0, 0, d, [i * (NB // 2) + g for g in range((NB + 1) // 2)], tok)
            jobs.insert(2 * d + 1, job_k)
        for n in range(4):
            def job_h(tok, n=n):
                build_kh(0, 0, [i * 64 + n * 16 + t for t in range(16)], tok)
            jobs.append(job_h)
        nside = 3 * (H // HG) - 1
        cnt = [0]

        def side(res):
            k = cnt[0]
            cnt[0] += 1
            mine = jobs[(k * len(jobs)) // nside:((k + 1) * len(jobs)) // nside] if k < nside else []
            for n, job in enumerate(mine):
                rr = (n * HG * DH // len(mine)) // 8 * 8
                job(res[rr:rr + 8, 0:128])

        qproj(2 * i, side)
        qproj(2 * i + 1, side)
        vproj(2 + i, None, side)
        return carry

    jax.lax.fori_loop(0, 2, qvloop, 0)

    def opaque_zero():
        state['cnt'] += 1
        return (state['h'] + state['cnt']) >> 20

    def vpu_block(h, par, i, tok):
        qt, c, j, t = BLIST[i]
        u = qt * NCK + c
        z0 = opaque_zero()
        qi = qt * H + h + z0
        row = lambda d: d if par == 0 else (d + 4) % 24
        lanes = slice(t * 128, (t + 1) * 128)
        acc = jnp.broadcast_to(qw_s[qi, row(DH):row(DH) + 1, lanes], (16, 128))
        for d in range(DH):
            kb = kbuf[par][GBASE[c] + j + z0, d]
            qb = qw_s[qi, row(d):row(d) + 1, lanes]
            if d == GATE:
                qb = gate(jnp.broadcast_to(qb, (8, 128)), tok)
                qb = jnp.concatenate([qb, qb], axis=0)
            acc = acc + kb * qb
        r0 = (CK - 16 * (j + 1)) // 2
        pbufs[u % NPB][r0:r0 + 8, lanes] = pltpu.bitcast(jnp.exp2(acc).astype(bf16), u32)

    def qk_unit(h, par, u):
        qt, c = divmod(u, NCK)
        nm = CK - 16 * NGRP[c]
        z0 = opaque_zero() * 8
        if not isinstance(z0, int):
            z0 = pl.multiple_of(z0, 8)
        kc = pltpu.bitcast(khbuf[par][pl.ds(c * (CK // 2) + z0, nm // 2), :], bf16)[:, 0:32]
        s = jnp.dot(kc, pltpu.bitcast(qm_s[qt * H + h], bf16), preferred_element_type=f32)
        pbufs[u % NPB][pl.ds(0, nm // 2), :] = pltpu.bitcast(jnp.exp2(s).astype(bf16), u32)
        return [s[r:r + 8, 0:128] for r in range(0, nm, 8)]

    def pv_unit(h, u, acc, zp):
        kc = (u % NCK) * CK
        p = pltpu.bitcast(pbufs[u % NPB][pl.ds(zp, 64), :], bf16)
        o = jnp.dot(vt_s[kc // RC, h, :, pl.ds(kc % RC, CK)], p, preferred_element_type=f32)
        return acc + o, [o[r:r + 8, 0:128] for r in range(0, 24, 8)]

    def ffn_piece(h, p, side):
        kind, j = p
        z0 = opaque_zero()
        acc = None
        for sidx in range(NSUB[kind]):
            if kind == 'gu':
                rows = pl.ds(pl.multiple_of((h + z0) * (FM // 2), FM // 2), FM // 2)
                a = pltpu.bitcast(xn_s[rows, sidx * 128:(sidx + 1) * 128], bf16)
                w = pltpu.bitcast(wgu_p[j, sidx * 64:(sidx + 1) * 64, :], bf16)
            else:
                a = pltpu.bitcast(hh_s[pl.ds(pl.multiple_of(z0 * 8, 8), FM // 2), sidx * 512:(sidx + 1) * 512], bf16)
                w = pltpu.bitcast(wd_p[j, sidx * 256:(sidx + 1) * 256, :], bf16)
            o = jnp.dot(a, w, preferred_element_type=f32)
            acc = o if acc is None else acc + o
            side(sidx * FT, [o[ti * (FM // FT):ti * (FM // FT) + 8, 0:128] for ti in range(FT)])
        if kind == 'gu':
            g = acc[:, :256]
            u = acc[:, 256:]
            hh = (g * u) * (0.5 * jnp.tanh(0.5 * g) + 0.5)
            hh_s[:, j * 256:(j + 1) * 256] = pltpu.bitcast(hh.astype(bf16), u32)
        else:
            y_s[pl.ds(pl.multiple_of(h * FM, FM), FM), j * 128:(j + 1) * 128] = acc

    def block(h, par):
        state['h'] = h
        state['neg'] = h >> 20
        zp = pl.multiple_of((h >> 20) * 8, 8)
        hp = jnp.maximum(h - 1, 0)
        hn = jnp.minimum(h + 1, H - 1)
        hn2 = jnp.minimum(h + 1, H - 1 - par)
        acc = acc_s[...]

        def side(k0, toks):
            for ti, tok in enumerate(toks):
                idxs = KASSIGN[k0 + ti]
                for d in sorted(set(i // NB for i in idxs)):
                    build_kb(hn, 1 - par, d, [i % NB for i in idxs if i // NB == d], tok)
                if HASSIGN[k0 + ti]:
                    build_kh(hn2, 1 - par, HASSIGN[k0 + ti], tok)
                for i in ASSIGN[k0 + ti]:
                    vpu_block(h, par, i, tok)

        for v in range(UPH):
            u = v - LEAD
            side(TOK0[(v, 'qk')], qk_unit(h, par, u) if u >= 0 else qk_unit(hp, 1 - par, u % UPH))
            w = u - LAGU
            hw = h if w >= 0 else hp
            qt, c = divmod(w % UPH, NCK)
            if c == 0:
                acc = zero_s[h >> 20]
            acc, toks = pv_unit(hw, w % UPH, acc, zp)
            side(TOK0[(v, 'pv')], toks)
            if c == NCK - 1:
                oraw_s[hw * NQ + qt] = acc
            if v in PPOS:
                ffn_piece(h, PPOS[v], lambda o, toks: side(TOK0[(v, 'ffn')] + o, toks))
        acc_s[...] = acc

    def body(b, carry):
        pl.when((b >> 20) == 0)(lambda: block(2 * b, 0))
        pl.when((b >> 21) == 0)(lambda: block(2 * b + 1, 1))
        return carry

    jax.lax.fori_loop(0, H // 2, body, 0)

    cp_wo.wait()
    state['h'] = 0
    for u in range(UPH - LEAD, UPH):
        qk_unit(H - 1, 1, u)
    acc = acc_s[...]
    for w in range(UPH - LEAD - LAGU, UPH):
        acc, _ = pv_unit(H - 1, w, acc, 0)
    oraw_s[H * NQ - 1] = acc

    def fallback():
        def item(it, carry):
            h = it // NQ
            qt = it % NQ
            odd = h % 2
            row24 = jax.lax.broadcasted_iota(i32, (24, TQ), 0)
            w = jnp.where(row24 == 20 - 20 * odd, 0.0, qw_s[qt * H + h])
            w = jnp.concatenate([w, jnp.zeros((8, TQ), f32)], axis=0).astype(bf16)
            sh = (4 * odd - DH * h) % 128

            def p1(c, m):
                kc = pltpu.roll(k_s[h // 6, pl.ds(pl.multiple_of(c * (CK // 2), CK // 2), CK // 2), :], sh, axis=1)
                s = jnp.dot(pltpu.bitcast(kc, bf16)[:, 0:32], w, preferred_element_type=f32)
                sfb_s[pl.ds(pl.multiple_of(c * CK, CK), CK), :] = s
                return jnp.maximum(m, jnp.max(s.reshape(CK // 8, 8, TQ), axis=0))
            m = jax.lax.fori_loop(0, NCK, p1, jnp.full((8, TQ), -jnp.inf, f32))
            m = jnp.max(m, axis=0, keepdims=True)

            def p2(r, acc):
                s = sfb_s[pl.ds(pl.multiple_of(r * RC, RC), RC), :]
                p = jnp.exp2(s - m).astype(bf16)
                return acc + jnp.dot(vt_s[r, h], p, preferred_element_type=f32)
            oraw_s[it] = jax.lax.fori_loop(0, NR, p2, jnp.zeros((24, TQ), f32))
            return carry
        jax.lax.fori_loop(0, H * NQ, item, 0)

    def out_copy(t):
        return pltpu.make_async_copy(out_s.at[pl.ds(t * TO, TO), :], o_hbm.at[pl.ds(t * TO, TO), :], sem_out.at[t])

    def tail(qt, carry):
        lo, hi = carry
        row8 = jax.lax.broadcasted_iota(i32, (8, TQ), 0)

        def bcast(ref_row):
            return jnp.concatenate([jnp.broadcast_to(ref_row(slice(n * 128, (n + 1) * 128)), (8, 128))
                                    for n in range(TQ // 128)], axis=1)

        pieces = []
        for g8 in range(H // 8):
            lst = None
            for k in range(8):
                h = g8 * 8 + k
                lrow = 20 if h % 2 == 0 else 0
                lk = bcast(lambda ln_: oraw_s[h * NQ + qt, lrow:lrow + 1, ln_])
                lst = lk if lst is None else jnp.where(row8 == k, lk, lst)
            lo = jnp.minimum(lo, lst)
            hi = jnp.maximum(hi, lst)
            rinv_s[g8 * 8:(g8 + 1) * 8, :] = 1.0 / lst
            for g in range(g8 * 4, g8 * 4 + 4):
                ra = bcast(lambda ln_: rinv_s[2 * g:2 * g + 1, ln_])
                rb = bcast(lambda ln_: rinv_s[2 * g + 1:2 * g + 2, ln_])
                a = oraw_s[2 * g * NQ + qt]
                b = oraw_s[(2 * g + 1) * NQ + qt]
                pieces += [a[0:8] * ra, a[8:16] * ra,
                           jnp.where(row8 < 4, a[16:24] * ra, b[0:8] * rb), b[8:16] * rb, b[16:24] * rb]
        ot = jnp.concatenate(pieces, axis=0).astype(bf16)
        for e in range(TQ // TO):
            rows = pl.ds(pl.multiple_of(qt * TQ + e * TO, TO), TO)
            acc = x_s[rows, :].astype(f32) + y_s[rows, :]
            acc = acc + jax.lax.dot_general(ot[:, e * TO:(e + 1) * TO], wo_s[...], (((0,), (0,)), ((), ())),
                                            preferred_element_type=f32)
            out_s[rows, :] = acc.astype(bf16)
            pltpu.make_async_copy(out_s.at[rows, :], o_hbm.at[rows, :], sem_out.at[qt * (TQ // TO) + e]).start()
        return lo, hi

    def one_pass(p, carry):
        @pl.when(jnp.logical_or(p == 0, flag_s[0] != 0))
        def _():
            lo, hi = jax.lax.fori_loop(0, NQ, tail, (jnp.ones((8, TQ), f32), jnp.ones((8, TQ), f32)))
            vm = jnp.maximum(jnp.max(vmax_s[...]), 1.0)
            ok = (lo >= L_MIN) & (hi * vm <= L_MAX)
            flag_s[0] = (jnp.max(jnp.where(ok, 0.0, 1.0)) > 0.0).astype(i32)
            for t in range(S // TO):
                out_copy(t).wait()
            pl.when(jnp.logical_and(p == 0, flag_s[0] != 0))(fallback)
        return carry

    jax.lax.fori_loop(0, 2, one_pass, 0)


@jax.jit
def pallas_parallel_sum__mha_block__swiglu_ffn__prompt_kernel(A_x, A_wqkv, A_wo, B_x, B_w_gate, B_w_up, B_w_down):
    x = A_x.reshape(S, D)
    bf16 = jnp.bfloat16
    f32 = jnp.float32
    u32 = jnp.uint32
    anyspec = pl.BlockSpec(memory_space=pl.ANY)
    out = pl.pallas_call(
        _kernel,
        in_specs=[anyspec] * 6,
        out_specs=anyspec,
        out_shape=jax.ShapeDtypeStruct((S, D), bf16),
        scratch_shapes=[
            pltpu.VMEM((S, D), bf16),
            pltpu.VMEM((D, D), bf16),
            pltpu.VMEM((D, D), bf16),
            pltpu.VMEM((D, D), bf16),
            pltpu.VMEM((D, D), bf16),
            pltpu.VMEM((D, F), bf16),
            pltpu.VMEM((D, F), bf16),
            pltpu.VMEM((F, D), bf16),
            pltpu.VMEM((S, D), bf16),
            pltpu.VMEM((S // 2, D), u32),
            pltpu.VMEM((2 * D, D), bf16),
            pltpu.VMEM((NSLAB, S // 2, 128), u32),
            pltpu.VMEM((NQ * H, 16, TQ), u32),
            pltpu.VMEM((NR, H, 24, RC), f32),
            pltpu.VMEM((H * NQ, 24, TQ), f32),
            pltpu.VMEM((H, NBA * 16, 128), f32),
            pltpu.VMEM((NQ * H, 24, TQ), f32),
            pltpu.VMEM((NBA, DH, 16, 128), f32),
            pltpu.VMEM((NBA, DH, 16, 128), f32),
            pltpu.VMEM((S // 2, 128), u32),
            pltpu.VMEM((S // 2, 128), u32),
            pltpu.VMEM((6, D // 2, 512), u32),
            pltpu.VMEM((5, F // 2, 128), u32),
            pltpu.VMEM((FM // 2, F), u32),
            pltpu.VMEM((S, D), f32),
            pltpu.VMEM((1, 24, TQ), f32),
            pltpu.VMEM((24, TQ), f32),
            pltpu.VMEM((H, 128), f32),
            pltpu.VMEM((8, RC), f32),
            pltpu.VMEM((H, TQ), f32),
            pltpu.SMEM((2,), jnp.int32),
            pltpu.VMEM((S, TQ), f32),
            pltpu.SemaphoreType.DMA((13,)),
            pltpu.SemaphoreType.DMA((S // TO,)),
        ] + [pltpu.VMEM((64, TQ), u32)] * NPB,
        compiler_params=pltpu.CompilerParams(
            vmem_limit_bytes=116 * 1024 * 1024),
        name="fused_block",
    )(x, A_wqkv, A_wo, B_w_gate, B_w_up, B_w_down)
    return out.reshape(1, S, D)
```

```python
import bisect

import jax
import jax.numpy as jnp
import jax.experimental.pallas as pl
import jax.experimental.pallas.tpu as pltpu

S = 2048
D = 640
H = 32
DH = 20
F = 1536
EPS = 1e-5
NSLAB = 6
LOG2E = 1.4426950408889634
SHIFT = 100.0
L_MIN = 2.0 ** -80
L_MAX = 2.0 ** 124

TQ = 512
CK = 128
NCK = S // CK
NQ = S // TQ
RC = 512
NR = S // RC
CPR = RC // CK
TO = 256
NB = 23
GATE = DH - 1
LAGU = 3
LEAD = 0
NPB = 8
FM = S // H
FT = 8
HG = 4

NBA = (NB + 2) // 2 * 2
NGRP = [((c + 1) * NB) // NCK - (c * NB) // NCK for c in range(NCK)]
GBASE = [(c * NB) // NCK for c in range(NCK)]
UPH = NQ * NCK
BLIST = [(qt, c, j, t) for qt in range(NQ) for c in range(NCK) for j in range(NGRP[c]) for t in range(4)]


def _plan():
    pieces = [('gu', j) for j in range(6)] + [('dn', n) for n in range(5)]
    nsub = {'gu': 5, 'dn': 3}
    ppos = {4 + (i * (UPH - 8)) // len(pieces): p for i, p in enumerate(pieces)}
    ttime, tunit, tok0 = [], [], {}
    t = 0
    for v in range(UPH):
        nm = CK - 16 * NGRP[(v - LEAD) % NCK]
        tok0[(v, 'qk')] = len(ttime)
        for ti in range(nm // 8):
            ttime.append(t + ti * 8)
            tunit.append(v)
        t += nm
        tok0[(v, 'pv')] = len(ttime)
        for ti in range(3):
            ttime.append(t + ti * 8)
            tunit.append(v + 1)
        t += 24
        if v in ppos:
            tok0[(v, 'ffn')] = len(ttime)
            for _ in range(nsub[ppos[v][0]]):
                for ti in range(FT):
                    ttime.append(t + ti * (FM // FT))
                    tunit.append(v + 1)
                t += FM
    assign = [[] for _ in ttime]
    kassign = [[] for _ in ttime]
    for i, (qt, c, _, _) in enumerate(BLIST):
        k = min(bisect.bisect_left(ttime, (i - 0.5) * t / len(BLIST)), len(ttime) - 1)
        assign[k].append(i)
        u = qt * NCK + c
        assert u - (NPB - LAGU - LEAD - 1) <= tunit[k] <= u + LEAD + LAGU - 1
    nk = DH * NB
    for i in range(nk):
        kassign[bisect.bisect_left(ttime, i * (t - 600) / nk)].append(i)
    hassign = [[] for _ in ttime]
    for i in range(len(HLIST)):
        hassign[bisect.bisect_left(ttime, 300 + (i // 2 * 2) * (t - 600) / len(HLIST))].append(HLIST[i])
    return ppos, nsub, tok0, assign, kassign, hassign


HLIST = [c * (CK // 16) + n for c in range(NCK) for n in range(CK // 16 - NGRP[c])]
PPOS, NSUB, TOK0, ASSIGN, KASSIGN, HASSIGN = _plan()


def _kernel(x_hbm, wqkv_hbm, wo_hbm, wg_hbm, wu_hbm, wd_hbm, o_hbm,
            x_s, wq_s, wk_s, wv_s, wo_s, wg_s, wu_s, wd_s, out_s,
            xn_s, wqvt_s, k_s, qm_s, vt_s, oraw_s, koff_s, qw_s, kb_a, kb_b, kh_a, kh_b,
            wgu_p, wd_p, hh_s, y_s, zero_s, acc_s, kcol_s, vmax_s, rinv_s, flag_s, sfb_s,
            sem_in, sem_out, *pbufs):
    f32 = jnp.float32
    bf16 = jnp.bfloat16
    u32 = jnp.uint32
    i32 = jnp.int32
    kbuf = (kb_a, kb_b)
    khbuf = (kh_a, kh_b)

    cp_x0 = pltpu.make_async_copy(x_hbm.at[pl.ds(0, RC), :], x_s.at[pl.ds(0, RC), :], sem_in.at[0])
    cp_wk = pltpu.make_async_copy(wqkv_hbm.at[:, pl.ds(D, D)], wk_s, sem_in.at[1])
    cp_wq = pltpu.make_async_copy(wqkv_hbm.at[:, pl.ds(0, D)], wq_s, sem_in.at[2])
    cp_wv = pltpu.make_async_copy(wqkv_hbm.at[:, pl.ds(2 * D, D)], wv_s, sem_in.at[3])
    cp_x1 = pltpu.make_async_copy(x_hbm.at[pl.ds(RC, RC), :], x_s.at[pl.ds(RC, RC), :], sem_in.at[4])
    cp_xr = pltpu.make_async_copy(x_hbm.at[pl.ds(2 * RC, 2 * RC), :], x_s.at[pl.ds(2 * RC, 2 * RC), :],
                                  sem_in.at[5])
    cp_wo = pltpu.make_async_copy(wo_hbm, wo_s, sem_in.at[6])

    def late(i):
        cps = []
        for n, (src, dst) in enumerate(((wg_hbm, wg_s), (wu_hbm, wu_s), (wd_hbm, wd_s))):
            hr = src.shape[0] // 2
            rows = pl.ds(i * hr if isinstance(i, int) else pl.multiple_of(i * hr, hr), hr)
            cps.append(pltpu.make_async_copy(src.at[rows, :], dst.at[rows, :], sem_in.at[7 + 3 * i + n]))
        return cps

    for c in (cp_x0, cp_wk, cp_wv, cp_x1, cp_xr, cp_wq):
        c.start()
    flag_s[0] = 0
    flag_s[1] = 0

    state = dict(h=0, cnt=0, neg=0)

    def gate(val, tok):
        r, c = val.shape
        mask = jax.lax.broadcasted_iota(i32, (r, c), 1) < state['neg']
        t = tok if val.dtype == tok.dtype else pltpu.bitcast(tok, val.dtype)
        t = jnp.concatenate([jnp.concatenate([t] * (c // 128), axis=1)] * (r // 8), axis=0)
        return jnp.where(mask, t, val)

    def xn_chunk(r):
        start = r * (RC // 2)
        if not isinstance(r, int):
            start = pl.multiple_of(start, RC // 2)
        return pltpu.bitcast(xn_s[pl.ds(start, RC // 2), :], bf16)

    def ln(r):
        x = x_s[pl.ds(r * RC, RC), :].astype(f32)
        mu = jnp.mean(x, axis=-1, keepdims=True)
        xc = x - mu
        var = jnp.mean(xc * xc, axis=-1, keepdims=True)
        xn_s[pl.ds(r * (RC // 2), RC // 2), :] = pltpu.bitcast((xc * jax.lax.rsqrt(var + EPS)).astype(bf16), u32)

    def ind_k():
        l = jax.lax.broadcasted_iota(i32, (D, 128), 0)
        h = jax.lax.broadcasted_iota(i32, (D, 128), 1)
        return jnp.where((l >= DH * h) & (l < DH * h + DH), 1.0, 0.0).astype(bf16)

    def kproj(r, kmax):
        kk = jnp.dot(xn_chunk(r), wk_s[...], preferred_element_type=f32)
        k2 = kk * kk
        k2 = jnp.maximum(k2[0:RC // 2], k2[RC // 2:RC]).astype(bf16)
        kn2 = jnp.dot(k2, ind_k(), preferred_element_type=f32)
        kn2 = jnp.max(kn2.reshape(RC // 16, 8, 128), axis=0)
        kmax = kn2 if kmax is None else jnp.maximum(kmax, kn2)
        lane = jax.lax.broadcasted_iota(i32, (RC, 128), 1)
        g0 = GBASE[r * CPR]
        for j in range(NSLAB):
            jt = min(j, 4)
            kj = kk[:, jt * 128:(jt + 1) * 128]
            if 1 <= j <= 4:
                kj = jnp.where(lane >= 128 - 8 * j, kk[:, (j - 1) * 128:j * 128], kj)
            kj = kj.astype(bf16)
            k_s[j, pl.ds(r * (RC // 2), RC // 2), :] = pltpu.bitcast(kj, u32)
            rows = []
            for cc in range(CPR):
                for g in range(NGRP[r * CPR + cc]):
                    a = cc * CK + CK - 16 * (g + 1)
                    rows.append(kj[a:a + 16, :])
            ko = jnp.concatenate(rows, axis=0).astype(f32)
            for h in range(6 * j, min(6 * j + 6, H)):
                lo = (DH * h) % 128
                koff_s[h, g0 * 16:(g0 + len(rows)) * 16, :] = pltpu.roll(ko, 128 - lo, axis=1) if lo else ko
        return kmax

    def qproj(r, side):
        xn = xn_chunk(r)
        mg = HG * DH
        row24 = jax.lax.broadcasted_iota(i32, (24, RC), 0)
        zpad = jnp.zeros((8, RC), f32)
        for gq in range(H // HG):
            qt = jax.lax.dot_general(wqvt_s[gq * mg:(gq + 1) * mg, :], xn, (((1,), (1,)), ((), ())),
                                     preferred_element_type=f32) * (DH ** -0.5 * LOG2E)
            side(qt)
            qr = qt.astype(bf16).astype(f32)
            for h in range(gq * HG, (gq + 1) * HG):
                base = (DH * h // 8) * 8 - gq * mg
                win = qr[base:base + 24, :]
                brow, v0 = (20, 0) if h % 2 == 0 else (0, 4)
                wm = jnp.where((row24 >= v0) & (row24 < v0 + DH), win, 0.0)
                qn2 = jnp.sum(wm * wm, axis=0, keepdims=True)
                kc = jnp.concatenate([kcol_s[h:h + 1, :]] * (RC // 128), axis=1)
                nbh = (SHIFT - jnp.sqrt(qn2 * kc) * 1.02).astype(bf16).astype(f32)
                wb = jnp.where(row24 == brow, nbh, wm)
                qw_s[r * H + h] = wb
                qm_s[r * H + h] = pltpu.bitcast(jnp.concatenate([wb, zpad], axis=0).astype(bf16), u32)

    def vproj(r, wvt=None, side=None, hg=HG):
        xn = xn_chunk(r)
        mg = hg * DH
        row24 = jax.lax.broadcasted_iota(i32, (24, RC), 0)
        for gq in range(H // hg):
            w = wqvt_s[D + gq * mg:D + (gq + 1) * mg, :] if wvt is None else wvt[gq * mg:(gq + 1) * mg, :]
            vt = jax.lax.dot_general(w, xn, (((1,), (1,)), ((), ())), preferred_element_type=f32)
            if side is not None:
                side(vt)
            vt = vt.astype(bf16).astype(f32)
            vmax_s[...] = jnp.maximum(vmax_s[...], jnp.max(jnp.abs(vt).reshape(mg // 8, 8, RC), axis=0))
            for h in range(gq * hg, (gq + 1) * hg):
                base = (DH * h // 8) * 8 - gq * mg
                ones_row = 20 if h % 2 == 0 else 0
                vt_s[r, h] = jnp.where(row24 == ones_row, 1.0, vt[base:base + 24, :])

    def build_kb(h, par, d, gs, tok):
        for g in gs:
            for half in range(2):
                st = g * 16 + half * 8
                ko = gate(koff_s[h, pl.ds(st if isinstance(st, int) else pl.multiple_of(st, 8), 8), :], tok)
                kbuf[par][g, d, half * 8:half * 8 + 8, :] = jnp.broadcast_to(ko[:, d:d + 1], (8, 128))

    def build_kh(h, par, tiles, tok):
        brow, v0 = (20, 0) if par == 0 else (0, 4)
        lane = jax.lax.broadcasted_iota(i32, (8, 128), 1)
        ones = gate(jnp.full((8, 128), 0x3F803F80, u32), tok)
        sh = (v0 - DH * h) % 128
        for t in tiles:
            rows = pl.ds(t * 8 if isinstance(t, int) else pl.multiple_of(t * 8, 8), 8)
            kt = k_s[h // 6, rows, :]
            if not (isinstance(sh, int) and sh == 0):
                kt = pltpu.roll(kt, sh, axis=1)
            khbuf[par][rows, :] = jnp.where(lane == brow, ones, kt)

    state['neg'] = flag_s[1]
    kh_b[...] = jnp.zeros(kh_b.shape, u32)
    zero_s[...] = jnp.zeros(zero_s.shape, f32)
    acc_s[...] = jnp.zeros(acc_s.shape, f32)
    vmax_s[...] = jnp.zeros(vmax_s.shape, f32)
    for pb in pbufs:
        pb[...] = jnp.zeros(pb.shape, u32)

    cp_x0.wait()
    ln(0)
    cp_wk.wait()
    kmax = kproj(0, None)
    cp_wv.wait()
    cp_x1.wait()
    for c in late(0) + late(1) + [cp_wo]:
        c.start()
    wvt = wv_s[...].T
    wqvt_s[D:2 * D, :] = wvt
    vproj(0, wvt, hg=16)
    ln(1)
    kmax = kproj(1, kmax)
    cp_xr.wait()
    cp_wq.wait()
    vproj(1, hg=16)
    ln(2)
    kmax = kproj(2, kmax)
    wqvt_s[0:D, :] = wq_s[...].T
    ln(3)
    kmax = kproj(3, kmax)
    krow = jnp.max(kmax, axis=0, keepdims=True)
    kcol_s[...] = jnp.broadcast_to(krow, (128, 128)).T[0:H, :]

    def qvloop(i, carry):
        for c in late(i):
            c.wait()
        jobs = []
        kr = pl.ds(pl.multiple_of(i * (D // 2), D // 2), D // 2)
        kr2 = pl.ds(pl.multiple_of(i * (D // 4), D // 4), D // 4)
        fr = pl.ds(pl.multiple_of(i * (F // 2), F // 2), F // 2)
        fr2 = pl.ds(pl.multiple_of(i * (F // 4), F // 4), F // 4)
        for j in range(12):
            def job_g(tok, j=j):
                o = (j % 2) * 128
                wgu_p[j // 2, kr2, o:o + 128] = gate(pltpu.bitcast(wg_s[kr, j * 128:(j + 1) * 128], u32), tok)

            def job_u(tok, j=j):
                o = 256 + (j % 2) * 128
                wgu_p[j // 2, kr2, o:o + 128] = gate(pltpu.bitcast(wu_s[kr, j * 128:(j + 1) * 128], u32), tok)
            jobs += [job_g, job_u]
        for n in range(5):
            def job_d(tok, n=n):
                wd_p[n, fr2, :] = gate(pltpu.bitcast(wd_s[fr, n * 128:(n + 1) * 128], u32), tok)
            jobs.append(job_d)
        for d in range(DH):
            def job_k(tok, d=d):
                build_kb(0, 0, d, [i * (NB // 2) + g for g in range((NB + 1) // 2)], tok)
            jobs.insert(2 * d + 1, job_k)
        for n in range(4):
            def job_h(tok, n=n):
                build_kh(0, 0, [i * 64 + n * 16 + t for t in range(16)], tok)
            jobs.append(job_h)
        nside = 3 * (H // HG) - 1
        cnt = [0]

        def side(res):
            k = cnt[0]
            cnt[0] += 1
            mine = jobs[(k * len(jobs)) // nside:((k + 1) * len(jobs)) // nside] if k < nside else []
            for n, job in enumerate(mine):
                rr = (n * HG * DH // len(mine)) // 8 * 8
                job(res[rr:rr + 8, 0:128])

        qproj(2 * i, side)
        qproj(2 * i + 1, side)
        vproj(2 + i, None, side)
        return carry

    jax.lax.fori_loop(0, 2, qvloop, 0)

    def opaque_zero():
        state['cnt'] += 1
        return (state['h'] + state['cnt']) >> 20

    def vpu_block(h, par, i, tok):
        qt, c, j, t = BLIST[i]
        u = qt * NCK + c
        z0 = opaque_zero()
        qi = qt * H + h + z0
        row = lambda d: d if par == 0 else (d + 4) % 24
        lanes = slice(t * 128, (t + 1) * 128)
        acc = jnp.broadcast_to(qw_s[qi, row(DH):row(DH) + 1, lanes], (16, 128))
        for d in range(DH):
            kb = kbuf[par][GBASE[c] + j + z0, d]
            qb = qw_s[qi, row(d):row(d) + 1, lanes]
            if d == GATE:
                qb = gate(jnp.broadcast_to(qb, (8, 128)), tok)
                qb = jnp.concatenate([qb, qb], axis=0)
            acc = acc + kb * qb
        r0 = (CK - 16 * (j + 1)) // 2
        pbufs[u % NPB][r0:r0 + 8, lanes] = pltpu.bitcast(jnp.exp2(acc).astype(bf16), u32)

    def qk_unit(h, par, u):
        qt, c = divmod(u, NCK)
        nm = CK - 16 * NGRP[c]
        z0 = opaque_zero() * 8
        if not isinstance(z0, int):
            z0 = pl.multiple_of(z0, 8)
        kc = pltpu.bitcast(khbuf[par][pl.ds(c * (CK // 2) + z0, nm // 2), :], bf16)[:, 0:32]
        s = jnp.dot(kc, pltpu.bitcast(qm_s[qt * H + h], bf16), preferred_element_type=f32)
        pbufs[u % NPB][pl.ds(0, nm // 2), :] = pltpu.bitcast(jnp.exp2(s).astype(bf16), u32)
        return [s[r:r + 8, 0:128] for r in range(0, nm, 8)]

    def pv_unit(h, u, acc, zp):
        kc = (u % NCK) * CK
        p = pltpu.bitcast(pbufs[u % NPB][pl.ds(zp, 64), :], bf16)
        o = jnp.dot(vt_s[kc // RC, h, :, pl.ds(kc % RC, CK)], p, preferred_element_type=f32)
        return acc + o, [o[r:r + 8, 0:128] for r in range(0, 24, 8)]

    def ffn_piece(h, p, side):
        kind, j = p
        z0 = opaque_zero()
        acc = None
        for sidx in range(NSUB[kind]):
            if kind == 'gu':
                rows = pl.ds(pl.multiple_of((h + z0) * (FM // 2), FM // 2), FM // 2)
                a = pltpu.bitcast(xn_s[rows, sidx * 128:(sidx + 1) * 128], bf16)
                w = pltpu.bitcast(wgu_p[j, sidx * 64:(sidx + 1) * 64, :], bf16)
            else:
                a = pltpu.bitcast(hh_s[pl.ds(pl.multiple_of(z0 * 8, 8), FM // 2), sidx * 512:(sidx + 1) * 512], bf16)
                w = pltpu.bitcast(wd_p[j, sidx * 256:(sidx + 1) * 256, :], bf16)
            o = jnp.dot(a, w, preferred_element_type=f32)
            acc = o if acc is None else acc + o
            side(sidx * FT, [o[ti * (FM // FT):ti * (FM // FT) + 8, 0:128] for ti in range(FT)])
        if kind == 'gu':
            g = acc[:, :256]
            u = acc[:, 256:]
            hh = (g * u) * (0.5 * jnp.tanh(0.5 * g) + 0.5)
            hh_s[:, j * 256:(j + 1) * 256] = pltpu.bitcast(hh.astype(bf16), u32)
        else:
            y_s[pl.ds(pl.multiple_of(h * FM, FM), FM), j * 128:(j + 1) * 128] = acc

    def block(h, par):
        state['h'] = h
        state['neg'] = h >> 20
        zp = pl.multiple_of((h >> 20) * 8, 8)
        hp = jnp.maximum(h - 1, 0)
        hn = jnp.minimum(h + 1, H - 1)
        hn2 = jnp.minimum(h + 1, H - 1 - par)
        acc = acc_s[...]

        def side(k0, toks):
            for ti, tok in enumerate(toks):
                idxs = KASSIGN[k0 + ti]
                if idxs:
                    koff_s[0, NB * 16:NB * 16 + 8, :] = tok
                    z8 = pl.multiple_of(opaque_zero() * 8, 8)
                    for i in idxs:
                        d, g = divmod(i, NB)
                        ko = koff_s[hn, pl.ds(g * 16 + z8, 16), :]
                        kbuf[1 - par][g, d] = jnp.broadcast_to(ko[:, d:d + 1], (16, 128))
                if HASSIGN[k0 + ti]:
                    build_kh(hn2, 1 - par, HASSIGN[k0 + ti], tok)
                for i in ASSIGN[k0 + ti]:
                    vpu_block(h, par, i, tok)

        for v in range(UPH):
            u = v - LEAD
            side(TOK0[(v, 'qk')], qk_unit(h, par, u) if u >= 0 else qk_unit(hp, 1 - par, u % UPH))
            w = u - LAGU
            hw = h if w >= 0 else hp
            qt, c = divmod(w % UPH, NCK)
            if c == 0:
                acc = zero_s[h >> 20]
            acc, toks = pv_unit(hw, w % UPH, acc, zp)
            side(TOK0[(v, 'pv')], toks)
            if c == NCK - 1:
                oraw_s[hw * NQ + qt] = acc
            if v in PPOS:
                ffn_piece(h, PPOS[v], lambda o, toks: side(TOK0[(v, 'ffn')] + o, toks))
        acc_s[...] = acc

    def body(b, carry):
        block(2 * b, 0)
        block(2 * b + 1, 1)
        return carry

    jax.lax.fori_loop(0, H // 2, body, 0)

    cp_wo.wait()
    state['h'] = 0
    for u in range(UPH - LEAD, UPH):
        qk_unit(H - 1, 1, u)
    acc = acc_s[...]
    for w in range(UPH - LEAD - LAGU, UPH):
        acc, _ = pv_unit(H - 1, w, acc, 0)
    oraw_s[H * NQ - 1] = acc

    def fallback():
        def item(it, carry):
            h = it // NQ
            qt = it % NQ
            odd = h % 2
            row24 = jax.lax.broadcasted_iota(i32, (24, TQ), 0)
            w = jnp.where(row24 == 20 - 20 * odd, 0.0, qw_s[qt * H + h])
            w = jnp.concatenate([w, jnp.zeros((8, TQ), f32)], axis=0).astype(bf16)
            sh = (4 * odd - DH * h) % 128

            def p1(c, m):
                kc = pltpu.roll(k_s[h // 6, pl.ds(pl.multiple_of(c * (CK // 2), CK // 2), CK // 2), :], sh, axis=1)
                s = jnp.dot(pltpu.bitcast(kc, bf16)[:, 0:32], w, preferred_element_type=f32)
                sfb_s[pl.ds(pl.multiple_of(c * CK, CK), CK), :] = s
                return jnp.maximum(m, jnp.max(s.reshape(CK // 8, 8, TQ), axis=0))
            m = jax.lax.fori_loop(0, NCK, p1, jnp.full((8, TQ), -jnp.inf, f32))
            m = jnp.max(m, axis=0, keepdims=True)

            def p2(r, acc):
                s = sfb_s[pl.ds(pl.multiple_of(r * RC, RC), RC), :]
                p = jnp.exp2(s - m).astype(bf16)
                return acc + jnp.dot(vt_s[r, h], p, preferred_element_type=f32)
            oraw_s[it] = jax.lax.fori_loop(0, NR, p2, jnp.zeros((24, TQ), f32))
            return carry
        jax.lax.fori_loop(0, H * NQ, item, 0)

    def out_copy(t):
        return pltpu.make_async_copy(out_s.at[pl.ds(t * TO, TO), :], o_hbm.at[pl.ds(t * TO, TO), :], sem_out.at[t])

    def tail(qt, carry):
        lo, hi = carry
        row8 = jax.lax.broadcasted_iota(i32, (8, TQ), 0)

        def bcast(ref_row):
            return jnp.concatenate([jnp.broadcast_to(ref_row(slice(n * 128, (n + 1) * 128)), (8, 128))
                                    for n in range(TQ // 128)], axis=1)

        pieces = []
        for g8 in range(H // 8):
            lst = None
            for k in range(8):
                h = g8 * 8 + k
                lrow = 20 if h % 2 == 0 else 0
                lk = bcast(lambda ln_: oraw_s[h * NQ + qt, lrow:lrow + 1, ln_])
                lst = lk if lst is None else jnp.where(row8 == k, lk, lst)
            lo = jnp.minimum(lo, lst)
            hi = jnp.maximum(hi, lst)
            rinv_s[g8 * 8:(g8 + 1) * 8, :] = 1.0 / lst
            for g in range(g8 * 4, g8 * 4 + 4):
                ra = bcast(lambda ln_: rinv_s[2 * g:2 * g + 1, ln_])
                rb = bcast(lambda ln_: rinv_s[2 * g + 1:2 * g + 2, ln_])
                a = oraw_s[2 * g * NQ + qt]
                b = oraw_s[(2 * g + 1) * NQ + qt]
                pieces += [a[0:8] * ra, a[8:16] * ra,
                           jnp.where(row8 < 4, a[16:24] * ra, b[0:8] * rb), b[8:16] * rb, b[16:24] * rb]
        ot = jnp.concatenate(pieces, axis=0).astype(bf16)
        for e in range(TQ // TO):
            rows = pl.ds(pl.multiple_of(qt * TQ + e * TO, TO), TO)
            acc = x_s[rows, :].astype(f32) + y_s[rows, :]
            acc = acc + jax.lax.dot_general(ot[:, e * TO:(e + 1) * TO], wo_s[...], (((0,), (0,)), ((), ())),
                                            preferred_element_type=f32)
            out_s[rows, :] = acc.astype(bf16)
            pltpu.make_async_copy(out_s.at[rows, :], o_hbm.at[rows, :], sem_out.at[qt * (TQ // TO) + e]).start()
        return lo, hi

    def one_pass(p, carry):
        @pl.when(jnp.logical_or(p == 0, flag_s[0] != 0))
        def _():
            lo, hi = jax.lax.fori_loop(0, NQ, tail, (jnp.ones((8, TQ), f32), jnp.ones((8, TQ), f32)))
            vm = jnp.maximum(jnp.max(vmax_s[...]), 1.0)
            ok = (lo >= L_MIN) & (hi * vm <= L_MAX)
            flag_s[0] = (jnp.max(jnp.where(ok, 0.0, 1.0)) > 0.0).astype(i32)
            for t in range(S // TO):
                out_copy(t).wait()
            pl.when(jnp.logical_and(p == 0, flag_s[0] != 0))(fallback)
        return carry

    jax.lax.fori_loop(0, 2, one_pass, 0)


@jax.jit
def pallas_parallel_sum__mha_block__swiglu_ffn__prompt_kernel(A_x, A_wqkv, A_wo, B_x, B_w_gate, B_w_up, B_w_down):
    x = A_x.reshape(S, D)
    bf16 = jnp.bfloat16
    f32 = jnp.float32
    u32 = jnp.uint32
    anyspec = pl.BlockSpec(memory_space=pl.ANY)
    out = pl.pallas_call(
        _kernel,
        in_specs=[anyspec] * 6,
        out_specs=anyspec,
        out_shape=jax.ShapeDtypeStruct((S, D), bf16),
        scratch_shapes=[
            pltpu.VMEM((S, D), bf16),
            pltpu.VMEM((D, D), bf16),
            pltpu.VMEM((D, D), bf16),
            pltpu.VMEM((D, D), bf16),
            pltpu.VMEM((D, D), bf16),
            pltpu.VMEM((D, F), bf16),
            pltpu.VMEM((D, F), bf16),
            pltpu.VMEM((F, D), bf16),
            pltpu.VMEM((S, D), bf16),
            pltpu.VMEM((S // 2, D), u32),
            pltpu.VMEM((2 * D, D), bf16),
            pltpu.VMEM((NSLAB, S // 2, 128), u32),
            pltpu.VMEM((NQ * H, 16, TQ), u32),
            pltpu.VMEM((NR, H, 24, RC), f32),
            pltpu.VMEM((H * NQ, 24, TQ), f32),
            pltpu.VMEM((H, NBA * 16, 128), f32),
            pltpu.VMEM((NQ * H, 24, TQ), f32),
            pltpu.VMEM((NBA, DH, 16, 128), f32),
            pltpu.VMEM((NBA, DH, 16, 128), f32),
            pltpu.VMEM((S // 2, 128), u32),
            pltpu.VMEM((S // 2, 128), u32),
            pltpu.VMEM((6, D // 2, 512), u32),
            pltpu.VMEM((5, F // 2, 128), u32),
            pltpu.VMEM((FM // 2, F), u32),
            pltpu.VMEM((S, D), f32),
            pltpu.VMEM((1, 24, TQ), f32),
            pltpu.VMEM((24, TQ), f32),
            pltpu.VMEM((H, 128), f32),
            pltpu.VMEM((8, RC), f32),
            pltpu.VMEM((H, TQ), f32),
            pltpu.SMEM((2,), jnp.int32),
            pltpu.VMEM((S, TQ), f32),
            pltpu.SemaphoreType.DMA((13,)),
            pltpu.SemaphoreType.DMA((S // TO,)),
        ] + [pltpu.VMEM((64, TQ), u32)] * NPB,
        compiler_params=pltpu.CompilerParams(
            vmem_limit_bytes=116 * 1024 * 1024),
        name="fused_block",
    )(x, A_wqkv, A_wo, B_w_gate, B_w_up, B_w_down)
    return out.reshape(1, S, D)
```
